```python
import jax
import jax.numpy as jnp

def _softmax(x, axis=-1):
    return jax.nn.softmax(x, axis=axis)

def _gelu(x):
    return jax.nn.gelu(x, approximate=True)

def _silu(x):
    return jax.nn.silu(x)

def _sigmoid(x):
    return jax.nn.sigmoid(x)

def _layernorm(x, axis=-1, eps=1e-05):
    m = jnp.mean(x, axis=axis, keepdims=True)
    v = jnp.var(x, axis=axis, keepdims=True)
    return (x - m) / jnp.sqrt(v + eps)

def _scatter_add(tgt, idx, src, axis=0):
    return tgt.at[idx].add(src)

def _segment_sum(src, seg, n):
    return jax.ops.segment_sum(src, seg, n)

class _Rng:

    def __init__(self, key):
        self._k = key

    def _next(self):
        self._k, sub = jax.random.split(self._k)
        return sub

    def normal(self, shape):
        return jax.random.normal(self._next(), shape, dtype=jnp.bfloat16)

    def randint(self, lo, hi, shape):
        return jax.random.randint(self._next(), shape, lo, hi, dtype=jnp.int32)

    def uniform(self, shape, lo=0.0, hi=1.0):
        return jax.random.uniform(self._next(), shape, jnp.bfloat16, lo, hi)

    def permutation(self, n):
        return jax.random.permutation(self._next(), n)
kernel_name = 'adaLN_cond__sliding_block_cached__moe_arch_mod__prompt'

def setup_inputs():
    _rng = _Rng(jax.random.key(int.from_bytes(__import__("os").urandom(4), "little")))
    _w = lambda a: (lambda t: t.astype(jnp.bfloat16) if jnp.issubdtype(t.dtype, jnp.floating) else t)(jnp.asarray(a))

    def _A_setup():
        B, Sq, D = (1, 2048, 1024)
        Hq, Hkv, Sk, Dh = (32, 4, 2048, 128)
        assert Hq % Hkv == 0, (Hq, Hkv)
        return {'x': _w((lambda *s: _rng.normal(s) * 0.05)(B, Sq, D)), 'k_cache': _w((lambda *s: _rng.normal(s) * 0.05)(B, Hkv, Sk, Dh)), 'v_cache': _w((lambda *s: _rng.normal(s) * 0.05)(B, Hkv, Sk, Dh)), 'wq': _w((lambda *s: _rng.normal(s) * 0.05)(D, Hq * Dh) * D ** (-0.5)), 'wo': _w((lambda *s: _rng.normal(s) * 0.05)(Hq * Dh, D) * (Hq * Dh) ** (-0.5))}
    _A_in = _A_setup()

    def _B_setup():
        B, S, D, F, C = (1, 2048, 1024, 3584, 1)
        return {'x': _w((lambda *s: _rng.normal(s) * 0.05)(B, S, D)), 'w_r': _w((lambda *s: _rng.normal(s) * 0.05)(D)), 'w_gate': _w((lambda *s: _rng.normal(s) * 0.05)(D, F)), 'w_up': _w((lambda *s: _rng.normal(s) * 0.05)(D, F)), 'w_down': _w((lambda *s: _rng.normal(s) * 0.05)(F, D))}
    _B_in = _B_setup()
    return {'A_x': _A_in['x'], 'A_k_cache': _A_in['k_cache'], 'A_v_cache': _A_in['v_cache'], 'A_wq': _A_in['wq'], 'A_wo': _A_in['wo'], 'B_x': _B_in['x'], 'B_w_r': _B_in['w_r'], 'B_w_gate': _B_in['w_gate'], 'B_w_up': _B_in['w_up'], 'B_w_down': _B_in['w_down'], 'c': _w((lambda *s: _rng.normal(s) * 0.05)(1, 1024)), 'w_mod': _w((lambda *s: _rng.normal(s) * 0.05)(1024, 6 * 1024) * 1024 ** (-0.5))}

def reference(A_x, A_k_cache, A_v_cache, A_wq, A_wo, B_x, B_w_r, B_w_gate, B_w_up, B_w_down, c, w_mod):

    def _A_ref(x, k_cache, v_cache, wq, wo):
        B, Sq, D = x.shape
        Hq, Dh = (32, 128)
        Hkv, Sk = (k_cache.shape[1], k_cache.shape[2])
        W = min(4096, max(256, Sk // 4))
        rep = Hq // Hkv
        q = (lambda x, *d: x.transpose(*d))((x @ wq).reshape(B, Sq, Hq, Dh), 0, 2, 1, 3)
        k = jnp.repeat(k_cache[:, :, Sk - W:, :], rep, axis=1)
        v = jnp.repeat(v_cache[:, :, Sk - W:, :], rep, axis=1)
        scores = jnp.einsum('bhqd,bhkd->bhqk', q, k) * Dh ** (-0.5)
        p = _softmax(scores, axis=-1)
        o = jnp.einsum('bhqk,bhkd->bhqd', p, v)
        return (lambda x, *d: x.transpose(*d))(o, 0, 2, 1, 3).reshape(B, Sq, Hq * Dh) @ wo

    def _B_ref(x, w_r, w_gate, w_up, w_down):
        B, S, D = x.shape
        C = 1
        r = x @ w_r
        idx = jnp.argsort(-r, axis=-1)[:, :C]
        idx_e = jnp.repeat(idx.reshape(B, C, 1), D, axis=2)
        x_sel = jnp.take_along_axis(x, idx_e, axis=1)
        g = _silu(x_sel @ w_gate)
        u = x_sel @ w_up
        y = g * u @ w_down
        r_sel = _sigmoid(jnp.take_along_axis(r, idx, axis=1))
        y = y * r_sel.reshape(B, C, 1)
        b_off = (jnp.arange(B) * S).reshape(B, 1)
        flat_idx = (idx + b_off).reshape(B * C)
        zero = (x * 0.0).reshape(B * S, D)
        upd = _scatter_add(zero, flat_idx, y.reshape(B * C, D), axis=0)
        return x + upd.reshape(B, S, D)
    x = A_x
    mod = (_silu(c) @ w_mod).reshape(c.shape[0], 6, 1, -1)
    sa, ca, ga, sb, cb, gb = (mod[:, 0].copy(), mod[:, 1].copy(), mod[:, 2].copy(), mod[:, 3].copy(), mod[:, 4].copy(), mod[:, 5].copy())
    h = _layernorm(x, axis=-1) * (1 + ca) + sa
    x = x + ga * _A_ref(h, A_k_cache, A_v_cache, A_wq, A_wo)
    h = _layernorm(x, axis=-1) * (1 + cb) + sb
    x = x + gb * _B_ref(h, B_w_r, B_w_gate, B_w_up, B_w_down)
    return x
```

```python
import contextlib
import functools
import numpy as np
import jax
import jax.numpy as jnp
from jax import lax
import jax.experimental.pallas as pl
import jax.experimental.pallas.tpu as pltpu

S, D, HQ, HKV, DH, SK, F = 2048, 1024, 32, 4, 128, 2048, 3584
W = 512
REP = HQ // HKV
GW = REP * DH
NP = D // 128
EPS = 1e-5
BF = jnp.bfloat16
F32 = jnp.float32
U32 = jnp.uint32
LOG2E = 1.4426950408889634
QSCALE = DH ** -0.5 * LOG2E


def _ln(xf, rel=None):
    m = jnp.sum(xf, axis=-1, keepdims=True)
    if rel is not None:
        m = m + rel
    m = m * (1.0 / D)
    d = xf - m
    v = jnp.sum(d * d, axis=-1, keepdims=True) * (1.0 / D)
    return d * lax.rsqrt(v + EPS)


def _recip(l):
    r = pl.reciprocal(l, approx=True)
    return r * (2.0 - l * r)


def make_kernel(TQ, scopes, opts):
    NT = S // TQ
    NS = NT * HKV
    CH = TQ // REP

    def scope(name):
        return jax.named_scope(name) if scopes else contextlib.nullcontext()

    def kernel(c_ref, wr_ref, x_hbm, k_hbm, v_hbm, wq_hbm, wo_hbm, wg_hbm, wu_hbm, wd_hbm, wm_hbm,
               out_hbm,
               x_v, k_v, v_v, kt_v, wq_v, wo_v, wg_v, wu_v, wd_v, wm_v, out_v, acc_v, h_v, x1_v, r_v,
               q_s, o_s, mod_v, zero_s, wr_s,
               sem_x, sem_kv, sem_wq, sem_wo, sem_ff, sem_wm, sem_out, sem_fin):
        mk = pltpu.make_async_copy

        def cp_x(t):
            r0 = t * TQ if isinstance(t, int) else pl.multiple_of(t * TQ, TQ)
            return [mk(x_hbm.at[pl.ds(r0, TQ)], x_v.at[pl.ds(r0, TQ)], sem_x.at[t])]

        def cp_wq(g, half=None):
            c0, n, s = (g * GW, GW, 2 * g) if half is None else (g * GW + half * (GW // 2), GW // 2, 2 * g + half)
            return [mk(wq_hbm.at[:, pl.ds(c0, n)], wq_v.at[:, pl.ds(c0, n)], sem_wq.at[s])]

        def cp_wo(g):
            return [mk(wo_hbm.at[pl.ds(g * GW, GW)], wo_v.at[pl.ds(g * GW, GW)], sem_wo.at[g])]

        def cp_kv(g):
            return [mk(k_hbm.at[g, pl.ds(SK - W, W), :], k_v.at[g], sem_kv.at[2 * g]),
                    mk(v_hbm.at[g, pl.ds(SK - W, W), :], v_v.at[g], sem_kv.at[2 * g + 1])]

        def cp_wm(ci):
            return [mk(wm_hbm.at[:, pl.ds(ci * 512, 512)], wm_v.at[:, pl.ds((ci * 512) % (4 * D), 512)], sem_wm.at[ci])]

        def cp_ff():
            return [mk(wg_hbm, wg_v, sem_ff.at[0]), mk(wu_hbm, wu_v, sem_ff.at[1]), mk(wd_hbm, wd_v, sem_ff.at[2])]

        def cp_out(t):
            r0 = t * TQ if isinstance(t, int) else pl.multiple_of(t * TQ, TQ)
            return [mk(out_v.at[pl.ds(r0, TQ)], out_hbm.at[pl.ds(r0, TQ)], sem_out.at[t])]

        def start(cps):
            for c_ in cps:
                c_.start()

        def wait(cps):
            for c_ in cps:
                c_.wait()

        def rows(r0, n):
            return pl.ds(r0 if isinstance(r0, int) else pl.multiple_of(r0, n), n)

        state = {"dead": [], "rel": None}

        def tok(v):
            if v.dtype == BF:
                u = pltpu.bitcast(v[0:16, 0:128], U32)
            else:
                u = pltpu.bitcast(v[0:8, 0:128], U32)
            return u & zero_s[...]

        def take_rel():
            z = state["rel"]
            if z is None:
                return None
            return jnp.concatenate([pltpu.bitcast(z, F32)[:, 0:1]] * (CH // 8), axis=0)

        def with_dead(lhs):
            if not state["dead"]:
                return lhs
            z = state["dead"][0]
            for z2 in state["dead"][1:]:
                z = z | z2
            state["dead"] = []
            n = lhs.shape[0]
            last = pltpu.bitcast(pltpu.bitcast(lhs[n - 16:n, :], U32) | z, BF)
            return jnp.concatenate([lhs[0:n - 16, :], last], axis=0)

        def reset_tokens():
            state["dead"] = []
            state["rel"] = None

        def mod_chunk(cs16, ci):
            c0 = (ci * 512) % (4 * D)
            m = jnp.dot(cs16, wm_v[:, c0:c0 + 512], preferred_element_type=F32)
            mod_v[:, ci * 512:(ci + 1) * 512] = m.astype(BF).astype(F32)

        def mod_row(which):
            return mod_v[0:1, which * D:(which + 1) * D]

        def one_plus(which):
            return (1 + mod_row(which).astype(BF)).astype(F32)

        def pre_chunk(t, ci):
            sl = rows(t * TQ + ci * CH, CH)
            xf = x_v[sl, :].astype(F32)
            h = (_ln(xf, take_rel()) * one_plus(1) + mod_row(0)).astype(BF)
            h_v[sl, :] = h
            state["dead"].append(tok(h[CH - 16:CH, D - 128:D]))

        def ln2(x1f, rel=None):
            return (_ln(x1f, rel) * one_plus(4) + mod_row(3)).astype(BF).astype(F32)

        def post_chunk(t, ci):
            sl = rows(t * TQ + ci * CH, CH)
            x1f = x1_v[sl, :].astype(F32)
            h2 = ln2(x1f, take_rel())
            r = jnp.sum(h2 * wr_s[...], axis=-1, keepdims=True).astype(BF).astype(F32)
            ob = (x1f + mod_row(5) * h2).astype(BF)
            out_v[sl, :] = ob
            r_v[sl, :] = jnp.broadcast_to(r, (CH, 128))
            state["dead"].append(tok(ob[CH - 16:CH, D - 128:D]) | tok(jnp.broadcast_to(r[CH - 8:CH, :], (8, 128))))

        def q_item(gq, tq, n, slot):
            c0 = gq * GW + n * DH
            if not isinstance(c0, int):
                c0 = pl.multiple_of(c0, DH)
            q = jnp.dot(h_v[rows(tq * TQ, TQ), :], wq_v[:, pl.ds(c0, DH)], preferred_element_type=F32)
            q_s[slot, n] = (q * QSCALE).astype(BF)

        def o_item(go, to, n, slot, fin, dead=False, rel=False):
            parts = [o_s[slot, k] for k in range(REP)]
            if dead:
                parts[0] = with_dead(parts[0])
            oo = jnp.concatenate(parts, axis=1)
            cs_ = slice(n * 128, (n + 1) * 128)
            part = jnp.dot(oo, wo_v[rows(go * GW, GW), cs_], preferred_element_type=F32)
            if rel:
                state["rel"] = tok(part)
            sl = rows(to * TQ, TQ)
            if fin:
                x1 = x_v[sl, cs_].astype(F32) + mod_v[0:1, 2 * D + n * 128:2 * D + (n + 1) * 128] * (acc_v[sl, cs_] + part)
                x1_v[sl, cs_] = x1.astype(BF)
            else:
                acc_v[sl, cs_] += part

        def s_item(g, hh, slot):
            qq = with_dead(q_s[slot, hh])
            return jnp.concatenate([jnp.dot(qq, kt_v[g, n], preferred_element_type=F32) for n in range(W // 128)], axis=1)

        def sm_item(s):
            m = jnp.max(s, axis=-1, keepdims=True)
            p = jnp.exp2(s - m)
            l = jnp.sum(p, axis=-1, keepdims=True)
            return p.astype(BF), _recip(l)

        def pv_item(g, hh, slot, p, rl):
            o = jnp.dot(p, v_v[g], preferred_element_type=F32)
            state["rel"] = tok(o)
            o_s[slot, hh] = (o * rl).astype(BF)

        def step(j, slot, do_q=True, do_o=True, fin=False, pre_t=None, post_t=None, post_t2=None):
            reset_tokens()
            g = j // NT
            gq, tq = (j + 1) // NT, (j + 1) % NT
            go, to = (j - 1) // NT, (j - 1) % NT
            s_next = s_item(g, 0, slot)
            for hh in range(REP):
                s_cur = s_next
                if hh + 1 < REP:
                    s_next = s_item(g, hh + 1, slot)
                if do_q:
                    q_item(gq, tq, hh, 1 - slot)
                if pre_t is not None:
                    pre_chunk(pre_t, hh)
                if post_t is not None:
                    post_chunk(post_t, hh)
                if post_t2 is not None:
                    post_chunk(post_t2, hh)
                p, rl = sm_item(s_cur)
                if do_o:
                    o_item(go, to, hh, 1 - slot, fin)
                pv_item(g, hh, slot, p, rl)

        def best_rows(r0, n):
            sub = lax.broadcasted_iota(jnp.int32, (8, 128), 0)
            items = [(r_v[r0 + i * 8:r0 + (i + 1) * 8, :], sub + (r0 + i * 8)) for i in range(n // 8)]
            while len(items) > 1:
                nxt = []
                for i in range(0, len(items) - 1, 2):
                    (av, ai), (bv_, bi_) = items[i], items[i + 1]
                    upd = bv_ > av
                    nxt.append((jnp.where(upd, bv_, av), jnp.where(upd, bi_, ai)))
                if len(items) % 2:
                    nxt.append(items[-1])
                items = nxt
            return items[0]

        with scope("prologue"):
            start(cp_x(0))
            for ci in range(4):
                start(cp_wm(ci))
            cs = c_ref[...].astype(F32)
            cs16 = jnp.broadcast_to((cs * jax.nn.sigmoid(cs)).astype(BF), (16, D))
            zero_s[...] = jnp.zeros((8, 128), U32)
            wr_s[...] = wr_ref[...].astype(F32).reshape(1, D)
            def zero_body(i, carry):
                acc_v[pl.ds(pl.multiple_of(i * 128, 128), 128), :] = jnp.zeros((128, D), F32)
                return carry
            lax.fori_loop(0, S // 128, zero_body, 0)
            x1_v[0:TQ, :] = jnp.zeros((TQ, D), BF)
            PV_ = opts.get("pv", 0)
            wait(cp_x(0))
            if PV_ == 0:
                start(cp_wq(0, 0)); start(cp_wq(0, 1)); start(cp_x(1)); start(cp_kv(0)); start(cp_x(2))
            for ci in range(4):
                wait(cp_wm(ci))
                if PV_ == 1 and ci == 1:
                    start(cp_wq(0, 0)); start(cp_x(1)); start(cp_kv(0)); start(cp_x(2)); start(cp_wq(0, 1))
                if PV_ == 2 and ci == 2:
                    start(cp_wq(0, 0)); start(cp_x(1)); start(cp_kv(0)); start(cp_x(2)); start(cp_wq(0, 1))
                if PV_ == 3 and ci == 2:
                    start(cp_wq(0, 0))
                if PV_ == 3 and ci == 3:
                    start(cp_wq(0, 1)); start(cp_x(1)); start(cp_kv(0)); start(cp_x(2))
                mod_chunk(cs16, ci)
            reset_tokens()
            for ci in range(REP):
                pre_chunk(0, ci)
            reset_tokens()
            wait(cp_wq(0, 0))
            start(cp_x(3))
            start(cp_x(4))
            start(cp_wo(0))
            for n in range(REP // 2):
                q_item(0, 0, n, 0)
            wait(cp_wq(0, 1))
            for t in range(5, NT):
                start(cp_x(t))
            for n in range(REP // 2, REP):
                q_item(0, 0, n, 0)
            wait(cp_x(1))
            for ci in range(REP):
                pre_chunk(1, ci)
            wait(cp_kv(0))
            for n in range(W // 128):
                kt_v[0, n] = k_v[0, n * 128:(n + 1) * 128, :].astype(F32).T.astype(BF)
            wait(cp_x(2))

        with scope("first"):
            step(0, 0, do_o=False, pre_t=2)
            wait(cp_wo(0))
            for g in range(1, HKV):
                start(cp_wq(g))
                start(cp_kv(g))
                start(cp_wo(g))
            for ci in range(4, 12):
                start(cp_wm(ci))
            start(cp_ff())

        def body_a0(i, carry):
            j = 2 * i + 1
            wait(cp_x(j + 2))

            @pl.when(j + 3 < NT)
            def _():
                wait(cp_x(j + 3))

            with scope("A0"):
                step(j, 1, pre_t=j + 2)
                step(j + 1, 0, pre_t=jnp.minimum(j + 3, NT - 1))
            return carry

        lax.fori_loop(0, NT // 2 - 1, body_a0, 0)

        with scope("mid"):
            for g in range(1, HKV):
                wait(cp_wq(g))
                wait(cp_kv(g))
                wait(cp_wo(g))
                for n in range(W // 128):
                    kt_v[g, n] = k_v[g, n * 128:(n + 1) * 128, :].astype(F32).T.astype(BF)

        def body_a1(i, carry):
            j = 2 * i + 1
            with scope("A1"):
                step(j, 1)
                step(j + 1, 0)
            return carry

        JB = (HKV - 1) * NT + 1
        lax.fori_loop(NT // 2 - 1, (JB - 1) // 2, body_a1, 0)

        with scope("modb"):
            for ci in range(4, 12):
                wait(cp_wm(ci))
            mb = jnp.dot(cs16, wm_v[:, 2 * D:4 * D], preferred_element_type=F32)
            mod_v[:, 2 * D:4 * D] = mb.astype(BF).astype(F32)
            mb = jnp.dot(cs16, wm_v[:, 0:2 * D], preferred_element_type=F32)
            mod_v[:, 4 * D:6 * D] = mb.astype(BF).astype(F32)

        def body_b(i, carry):
            j = 2 * i + 1
            with scope("B"):
                step(j, 1, fin=True, post_t=jnp.maximum(j - JB - 1, 0))
                step(j + 1, 0, fin=True, post_t=j - JB)

                @pl.when(j > JB)
                def _():
                    start(cp_out(j - JB - 1))
                start(cp_out(j - JB))
            return carry

        lax.fori_loop((JB - 1) // 2, (NS - 2) // 2, body_b, 0)

        with scope("last"):
            FD = opts.get("fd", 1)
            if FD == 5:
                step(NS - 1, 1, do_q=False, fin=True, post_t=NT - 3, post_t2=NT - 2)
            else:
                step(NS - 1, 1, do_q=False, fin=True, post_t=NT - 3)
            start(cp_out(NT - 3))
            reset_tokens()
            for n in range(NP):
                if FD == 0:
                    o_item(HKV - 1, NT - 1, n, 1, True, dead=True, rel=True)
                    post_chunk(NT - 2, n)
                elif FD == 1:
                    o_item(HKV - 1, NT - 1, n, 1, True)
                    post_chunk(NT - 2, n)
                    reset_tokens()
                elif FD == 2:
                    o_item(HKV - 1, NT - 1, n, 1, True, dead=True)
                    post_chunk(NT - 2, n)
                elif FD == 3:
                    held = state["dead"][-1:]
                    state["dead"] = state["dead"][:-1]
                    o_item(HKV - 1, NT - 1, n, 1, True, dead=True)
                    state["dead"] = held + state["dead"]
                    post_chunk(NT - 2, n)
                elif FD == 4:
                    held = state["dead"][-1:]
                    state["dead"] = state["dead"][:-1]
                    o_item(HKV - 1, NT - 1, n, 1, True, dead=True, rel=True)
                    state["dead"] = held + state["dead"]
                    post_chunk(NT - 2, n)
                elif FD == 5:
                    o_item(HKV - 1, NT - 1, n, 1, True)
            start(cp_out(NT - 2))
            av, ai = best_rows(0, (NT - 1) * TQ)
            reset_tokens()
            for ci in range(REP):
                post_chunk(NT - 1, ci)
            start(cp_out(NT - 1))
            bv_, bi_ = best_rows((NT - 1) * TQ, TQ)
            upd = bv_ > av
            bv, bi = jnp.where(upd, bv_, av), jnp.where(upd, bi_, ai)

        with scope("tail"):
            rmax = jnp.max(bv, axis=0, keepdims=True)
            idx = jnp.min(jnp.where(bv == rmax, bi, S))
            base = pl.multiple_of((idx // 16) * 16, 16)
            x1g = x1_v[pl.ds(base, 16), :].astype(F32)
            h2f = ln2(x1g)
            h2g = h2f.astype(BF)
            wait(cp_ff())
            acts = []
            for n in range(F // 128):
                fs = slice(n * 128, (n + 1) * 128)
                gt = jnp.dot(h2g, wg_v[:, fs], preferred_element_type=F32).astype(BF).astype(F32)
                up = jnp.dot(h2g, wu_v[:, fs], preferred_element_type=F32).astype(BF).astype(F32)
                acts.append(((gt * jax.nn.sigmoid(gt)).astype(BF).astype(F32) * up).astype(BF))
            ys = [jnp.dot(acts[n], wd_v[n * 128:(n + 1) * 128, :], preferred_element_type=F32) for n in range(F // 128)]
            while len(ys) > 1:
                ys = [ys[i] + ys[i + 1] if i + 1 < len(ys) else ys[i] for i in range(0, len(ys), 2)]
            y = ys[0].astype(BF).astype(F32)
            rs = jax.nn.sigmoid(rmax[:, 0:1]).astype(BF).astype(F32)
            y = (y * rs).astype(BF).astype(F32)
            sel = lax.broadcasted_iota(jnp.int32, (16, 1), 0) == (idx - base)
            hb = jnp.where(sel, (h2f + y).astype(BF).astype(F32), h2f)
            og = (x1g + mod_row(5) * hb).astype(BF)
            for t in range(NT):
                wait(cp_out(t))
            out_v[pl.ds(base, 16), :] = og
            fin = mk(out_v.at[pl.ds(base, 16)], out_hbm.at[pl.ds(base, 16)], sem_fin.at[0])
            fin.start()
            fin.wait()

    return kernel


def build(TQ=128, vmem_mb=110, scopes=False, **opts):
    NT = S // TQ

    @jax.jit
    def fn(A_x, A_k_cache, A_v_cache, A_wq, A_wo, B_x, B_w_r, B_w_gate, B_w_up, B_w_down, c, w_mod):
        x = A_x.reshape(S, D)
        k = A_k_cache.reshape(HKV, SK, DH)
        v = A_v_cache.reshape(HKV, SK, DH)
        wr = B_w_r
        any_spec = pl.BlockSpec(memory_space=pl.ANY)
        vm = pl.BlockSpec(memory_space=pltpu.VMEM)
        out = pl.pallas_call(
            make_kernel(TQ, scopes, opts),
            out_shape=jax.ShapeDtypeStruct((S, D), BF),
            in_specs=[vm, vm] + [any_spec] * 9,
            out_specs=any_spec,
            scratch_shapes=[
                pltpu.VMEM((S, D), BF),
                pltpu.VMEM((HKV, W, DH), BF),
                pltpu.VMEM((HKV, W, DH), BF),
                pltpu.VMEM((HKV, W // 128, DH, 128), BF),
                pltpu.VMEM((D, HQ * DH), BF),
                pltpu.VMEM((HQ * DH, D), BF),
                pltpu.VMEM((D, F), BF),
                pltpu.VMEM((D, F), BF),
                pltpu.VMEM((F, D), BF),
                pltpu.VMEM((D, 4 * D), BF),
                pltpu.VMEM((S, D), BF),
                pltpu.VMEM((S, D), F32),
                pltpu.VMEM((S, D), BF),
                pltpu.VMEM((S, D), BF),
                pltpu.VMEM((S, 128), F32),
                pltpu.VMEM((2, REP, TQ, DH), BF),
                pltpu.VMEM((2, REP, TQ, DH), BF),
                pltpu.VMEM((16, 6 * D), F32),
                pltpu.VMEM((8, 128), U32),
                pltpu.VMEM((1, D), F32),
                pltpu.SemaphoreType.DMA((NT,)),
                pltpu.SemaphoreType.DMA((2 * HKV,)),
                pltpu.SemaphoreType.DMA((2 * HKV,)),
                pltpu.SemaphoreType.DMA((HKV,)),
                pltpu.SemaphoreType.DMA((3,)),
                pltpu.SemaphoreType.DMA((12,)),
                pltpu.SemaphoreType.DMA((NT,)),
                pltpu.SemaphoreType.DMA((1,)),
            ],
            compiler_params=pltpu.CompilerParams(vmem_limit_bytes=vmem_mb * 1024 * 1024),
        )(c, wr, x, k, v, A_wq, A_wo, B_w_gate, B_w_up, B_w_down, w_mod)
        return out.reshape(1, S, D)

    return fn


_IMPL = build()


@jax.jit
def pallas_adaLN_cond__sliding_block_cached__moe_arch_mod__prompt_kernel(
    A_x: jax.Array,
    A_k_cache: jax.Array,
    A_v_cache: jax.Array,
    A_wq: jax.Array,
    A_wo: jax.Array,
    B_x: jax.Array,
    B_w_r: jax.Array,
    B_w_gate: jax.Array,
    B_w_up: jax.Array,
    B_w_down: jax.Array,
    c: jax.Array,
    w_mod: jax.Array,
):
    return _IMPL(A_x, A_k_cache, A_v_cache, A_wq, A_wo, B_x, B_w_r, B_w_gate, B_w_up, B_w_down, c, w_mod)
```

```python
import contextlib

import jax
import jax.numpy as jnp
from jax import lax
import jax.experimental.pallas as pl
import jax.experimental.pallas.tpu as pltpu

S, D, HQ, HKV, DH, SK, F = 2048, 1024, 32, 4, 128, 2048, 3584
W = min(4096, max(256, SK // 4))
REP = HQ // HKV
GW = REP * DH
NP = D // 128
TQ = 128
NT = S // TQ
NS = NT * HKV
CH = TQ // REP
EPS = 1e-5
BF = jnp.bfloat16
F32 = jnp.float32
U32 = jnp.uint32
LOG2E = 1.4426950408889634
QSCALE = DH ** -0.5 * LOG2E


def _ln(xf, rel=None):
    m = jnp.sum(xf, axis=-1, keepdims=True)
    if rel is not None:
        m = m + rel
    m = m * (1.0 / D)
    d = xf - m
    v = jnp.sum(d * d, axis=-1, keepdims=True) * (1.0 / D)
    return d * lax.rsqrt(v + EPS)


def _recip(l):
    r = pl.reciprocal(l, approx=True)
    return r * (2.0 - l * r)


def _tree_sum(xs):
    while len(xs) > 1:
        xs = [xs[i] + xs[i + 1] if i + 1 < len(xs) else xs[i] for i in range(0, len(xs), 2)]
    return xs[0]


def _make_kernel(scopes, opts):
    NTMM = opts.get("nt", False)
    POST_DL = opts.get("pdl", 1)

    def scope(name):
        return jax.named_scope(name) if scopes else contextlib.nullcontext()

    def kernel(c_ref, wr_ref, x_hbm, k_hbm, v_hbm, wq_hbm, wo_hbm, wg_hbm, wu_hbm, wd_hbm, wm_hbm,
               out_hbm,
               x_v, k_v, v_v, kt_v, wq_v, wo_v, wg_v, wu_v, wd_v, wm_v, out_v, acc_v, h_v, r_v,
               q_s, o_s, mod_v, zero_s, wr_s,
               sem_x, sem_wm, sem_g0, sem_rest, sem_out):
        mk = pltpu.make_async_copy

        def cp_x(t0, n, s):
            return [mk(x_hbm.at[pl.ds(t0 * TQ, n * TQ)], x_v.at[pl.ds(t0 * TQ, n * TQ)], sem_x.at[s])]

        def cp_wm(c0, n, s):
            return [mk(wm_hbm.at[:, pl.ds(c0, n)], wm_v.at[:, pl.ds(c0 % (4 * D), n)], sem_wm.at[s])]

        def cp_wq0(half):
            c0 = half * (GW // 2)
            return [mk(wq_hbm.at[:, pl.ds(c0, GW // 2)], wq_v.at[:, pl.ds(c0, GW // 2)], sem_g0.at[half])]

        def cp_kv0():
            return [mk(k_hbm.at[0, pl.ds(SK - W, W), :], k_v.at[0], sem_g0.at[2]),
                    mk(v_hbm.at[0, pl.ds(SK - W, W), :], v_v.at[0], sem_g0.at[3])]

        def cp_wo0():
            return [mk(wo_hbm.at[pl.ds(0, GW)], wo_v.at[pl.ds(0, GW)], sem_g0.at[4])]

        def cp_rest():
            n = HKV - 1
            return [mk(wq_hbm.at[:, pl.ds(GW, n * GW)], wq_v.at[:, pl.ds(GW, n * GW)], sem_rest.at[0]),
                    mk(wo_hbm.at[pl.ds(GW, n * GW)], wo_v.at[pl.ds(GW, n * GW)], sem_rest.at[0]),
                    mk(k_hbm.at[pl.ds(1, n), pl.ds(SK - W, W), :], k_v.at[pl.ds(1, n)], sem_rest.at[0]),
                    mk(v_hbm.at[pl.ds(1, n), pl.ds(SK - W, W), :], v_v.at[pl.ds(1, n)], sem_rest.at[0])]

        def cp_wm_b():
            return cp_wm(2 * D, 2 * D, 4) + cp_wm(4 * D, 2 * D, 4)

        def cp_ff():
            return [mk(wg_hbm, wg_v, sem_rest.at[1]), mk(wu_hbm, wu_v, sem_rest.at[1]), mk(wd_hbm, wd_v, sem_rest.at[1])]

        def cp_out(t):
            r0 = t * TQ if isinstance(t, int) else pl.multiple_of(t * TQ, TQ)
            return [mk(out_v.at[pl.ds(r0, TQ)], out_hbm.at[pl.ds(r0, TQ)], sem_out.at[0])]

        def start(cps):
            for cp in cps:
                cp.start()

        def wait(cps):
            for cp in cps:
                cp.wait()

        def rows(r0, n):
            return pl.ds(r0 if isinstance(r0, int) else pl.multiple_of(r0, n), n)

        state = {"dead": [], "rel": None}

        def tok(v):
            u = pltpu.bitcast(v[0:16, 0:128] if v.dtype == BF else v[0:8, 0:128], U32)
            return u & zero_s[...]

        def take_rel():
            if state["rel"] is None:
                return None
            return jnp.concatenate([pltpu.bitcast(state["rel"], F32)[:, 0:1]] * (CH // 8), axis=0)

        def with_dead(lhs):
            ready = [z for (z, n) in state["dead"] if n <= 0]
            state["dead"] = [(z, n - 1) for (z, n) in state["dead"] if n > 0]
            if not ready:
                return lhs
            z = ready[0]
            for z2 in ready[1:]:
                z = z | z2
            n = lhs.shape[0]
            last = pltpu.bitcast(pltpu.bitcast(lhs[n - 16:n, :], U32) | z, BF)
            return jnp.concatenate([lhs[0:n - 16, :], last], axis=0)

        def reset_tokens():
            state["dead"] = []
            state["rel"] = None

        def cs_dot(cs16, c0, n):
            ps = [jnp.dot(cs16[:, k * 128:(k + 1) * 128], wm_v[k * 128:(k + 1) * 128, c0:c0 + n],
                          preferred_element_type=F32) for k in range(NP)]
            return _tree_sum(ps).astype(BF).astype(F32)

        def mod_row(which):
            return mod_v[0:1, which * D:(which + 1) * D]

        def one_plus(which):
            return (1 + mod_row(which).astype(BF)).astype(F32)

        def pre_chunk(t, ci):
            sl = rows(t * TQ + ci * CH, CH)
            h = (_ln(x_v[sl, :].astype(F32), take_rel()) * one_plus(1) + mod_row(0)).astype(BF)
            h_v[sl, :] = h
            state["dead"].append((tok(h[CH - 16:CH, D - 128:D]), 0))

        def ln2(x1, rel=None):
            return _ln(x1, rel) * one_plus(4) + mod_row(3)

        def post_chunk(t, ci):
            sl = rows(t * TQ + ci * CH, CH)
            x1 = acc_v[sl, :]
            h2 = ln2(x1, take_rel())
            r = jnp.sum(h2 * wr_s[...], axis=-1, keepdims=True).astype(BF).astype(F32)
            ob = (x1 + mod_row(5) * h2).astype(BF)
            out_v[sl, :] = ob
            r_v[sl, :] = jnp.broadcast_to(r, (CH, 128))
            state["dead"].append((tok(ob[CH - 16:CH, D - 128:D]) | tok(jnp.broadcast_to(r[CH - 8:CH, :], (8, 128))), POST_DL))

        def q_item(gq, tq, n, slot):
            c0 = gq * GW + n * DH
            if not isinstance(c0, int):
                c0 = pl.multiple_of(c0, DH)
            q = jnp.dot(h_v[rows(tq * TQ, TQ), :], wq_v[:, pl.ds(c0, DH)], preferred_element_type=F32)
            q_s[slot, n] = (q * QSCALE).astype(BF)

        def o_item(go, to, n, slot, fin):
            oo = jnp.concatenate([o_s[slot, k] for k in range(REP)], axis=1)
            cs_ = slice(n * 128, (n + 1) * 128)
            part = jnp.dot(oo, wo_v[rows(go * GW, GW), cs_], preferred_element_type=F32)
            sl = rows(to * TQ, TQ)
            if fin:
                ga = mod_v[0:1, 2 * D + n * 128:2 * D + (n + 1) * 128]
                acc_v[sl, cs_] = x_v[sl, cs_].astype(F32) + ga * (acc_v[sl, cs_] + part)
            else:
                acc_v[sl, cs_] += part

        def s_item(g, hh, slot):
            qq = with_dead(q_s[slot, hh])
            if NTMM:
                return lax.dot_general(qq, k_v[g], (((1,), (1,)), ((), ())), preferred_element_type=F32)
            return jnp.concatenate([jnp.dot(qq, kt_v[g, n], preferred_element_type=F32)
                                    for n in range(W // 128)], axis=1)

        def softmax_item(s):
            m = jnp.max(s, axis=-1, keepdims=True)
            p = jnp.exp2(s - m)
            l = jnp.sum(p, axis=-1, keepdims=True)
            return p.astype(BF), _recip(l)

        def pv_item(g, hh, slot, p, rl):
            o = jnp.dot(p, v_v[g], preferred_element_type=F32)
            state["rel"] = tok(o)
            o_s[slot, hh] = (o * rl).astype(BF)

        def step(j, slot, do_q=True, do_o=True, fin=False, pre_t=None, post_t=None):
            g = j // NT
            gq, tq = (j + 1) // NT, (j + 1) % NT
            go, to = (j - 1) // NT, (j - 1) % NT
            s_next = s_item(g, 0, slot)
            for hh in range(REP):
                s_cur = s_next
                if hh + 1 < REP:
                    s_next = s_item(g, hh + 1, slot)
                if do_q:
                    q_item(gq, tq, hh, 1 - slot)
                if pre_t is not None:
                    pre_chunk(pre_t, hh)
                if post_t is not None:
                    post_chunk(post_t, hh)
                p, rl = softmax_item(s_cur)
                if do_o:
                    o_item(go, to, hh, 1 - slot, fin)
                pv_item(g, hh, slot, p, rl)

        def transpose_k(g):
            if not NTMM:
                for n in range(W // 128):
                    kt_v[g, n] = k_v[g, n * 128:(n + 1) * 128, :].astype(F32).T.astype(BF)

        def best_rows(r0, n):
            sub = lax.broadcasted_iota(jnp.int32, (8, 128), 0)
            items = [(r_v[r0 + i * 8:r0 + (i + 1) * 8, :], sub + (r0 + i * 8)) for i in range(n // 8)]
            while len(items) > 1:
                nxt = []
                for i in range(0, len(items) - 1, 2):
                    (av, ai), (bv, bi) = items[i], items[i + 1]
                    upd = bv > av
                    nxt.append((jnp.where(upd, bv, av), jnp.where(upd, bi, ai)))
                if len(items) % 2:
                    nxt.append(items[-1])
                items = nxt
            return items[0]

        with scope("prologue"):
            start(cp_x(0, 1, 0))
            for ci in range(4):
                start(cp_wm(ci * 512, 512, ci))
            cs = c_ref[...].astype(F32)
            cs16 = jnp.broadcast_to((cs * jax.nn.sigmoid(cs)).astype(BF), (16, D))
            zero_s[...] = jnp.zeros((8, 128), U32)
            wr_s[...] = wr_ref[...].astype(F32).reshape(1, D)

            def zero_body(i, carry):
                acc_v[pl.ds(pl.multiple_of(i * 128, 128), 128), :] = jnp.zeros((128, D), F32)
                return carry
            lax.fori_loop(0, S // 128, zero_body, 0)
            wait(cp_x(0, 1, 0))
            start(cp_wq0(0))
            start(cp_wq0(1))
            start(cp_x(1, 1, 1))
            start(cp_kv0())
            start(cp_x(2, 1, 2))
            for ci in range(4):
                wait(cp_wm(ci * 512, 512, ci))
                mod_v[:, ci * 512:(ci + 1) * 512] = cs_dot(cs16, ci * 512, 512)
            reset_tokens()
            for ci in range(REP):
                pre_chunk(0, ci)
            reset_tokens()
            wait(cp_wq0(0))
            start(cp_x(3, 2, 3))
            start(cp_wo0())
            for n in range(REP // 2):
                q_item(0, 0, n, 0)
            wait(cp_wq0(1))
            start(cp_x(5, NT - 5, 4))
            for n in range(REP // 2, REP):
                q_item(0, 0, n, 0)
            wait(cp_x(1, 1, 1))
            for ci in range(REP):
                pre_chunk(1, ci)
            wait(cp_kv0())
            transpose_k(0)
            wait(cp_x(2, 1, 2))

        with scope("first"):
            reset_tokens()
            step(0, 0, do_o=False, pre_t=2)
            wait(cp_wo0())
            wait(cp_x(3, 2, 3))
            start(cp_rest())
            start(cp_wm_b())
            start(cp_ff())

        def body_a0(i, carry):
            j = 2 * i + 1

            @pl.when(i == 1)
            def _():
                wait(cp_x(5, NT - 5, 4))

            reset_tokens()
            with scope("A0"):
                step(j, 1, pre_t=j + 2)
                step(j + 1, 0, pre_t=jnp.minimum(j + 3, NT - 1))
            return carry

        lax.fori_loop(0, NT // 2 - 1, body_a0, 0)

        with scope("mid"):
            wait(cp_rest())
            for g in range(1, HKV):
                transpose_k(g)

        def body_a1(i, carry):
            j = 2 * i + 1
            reset_tokens()
            with scope("A1"):
                step(j, 1)
                step(j + 1, 0)
            return carry

        JB = (HKV - 1) * NT + 1
        lax.fori_loop(NT // 2 - 1, (JB - 1) // 2, body_a1, 0)

        with scope("modb"):
            wait(cp_wm_b())
            mod_v[:, 2 * D:4 * D] = cs_dot(cs16, 2 * D, 2 * D)
            mod_v[:, 4 * D:6 * D] = cs_dot(cs16, 0, 2 * D)

        def body_b(i, carry):
            j = 2 * i + 1
            t = j - JB - 1
            reset_tokens()
            with scope("B"):
                step(j, 1, fin=True, post_t=jnp.maximum(t, 0))
                step(j + 1, 0, fin=True, post_t=t + 1)

                @pl.when(t >= 0)
                def _():
                    start(cp_out(t))
                start(cp_out(t + 1))
            return carry

        lax.fori_loop((JB - 1) // 2, (NS - 2) // 2, body_b, 0)

        with scope("last"):
            reset_tokens()
            step(NS - 1, 1, do_q=False, fin=True, post_t=NT - 3)
            start(cp_out(NT - 3))
            for n in range(NP):
                reset_tokens()
                o_item(HKV - 1, NT - 1, n, 1, True)
                post_chunk(NT - 2, n)
            start(cp_out(NT - 2))
            av, ai = best_rows(0, (NT - 1) * TQ)
            reset_tokens()
            for ci in range(REP):
                post_chunk(NT - 1, ci)
            start(cp_out(NT - 1))
            bv, bi = best_rows((NT - 1) * TQ, TQ)
            upd = bv > av
            bv, bi = jnp.where(upd, bv, av), jnp.where(upd, bi, ai)

        with scope("tail"):
            rmax = jnp.max(bv, axis=0, keepdims=True)
            idx = jnp.minimum(jnp.min(jnp.where(bv == rmax, bi, S)), S - 1)
            base = pl.multiple_of((idx // 16) * 16, 16)
            x1g = acc_v[pl.ds(base, 16), :]
            h2f = ln2(x1g)
            h2g = h2f.astype(BF)
            wait(cp_ff())
            acts = []
            for n in range(F // 128):
                fs = slice(n * 128, (n + 1) * 128)
                gt = jnp.dot(h2g, wg_v[:, fs], preferred_element_type=F32).astype(BF).astype(F32)
                up = jnp.dot(h2g, wu_v[:, fs], preferred_element_type=F32).astype(BF).astype(F32)
                acts.append(((gt * jax.nn.sigmoid(gt)).astype(BF).astype(F32) * up).astype(BF))
            ys = [jnp.dot(acts[n], wd_v[n * 128:(n + 1) * 128, :], preferred_element_type=F32)
                  for n in range(F // 128)]
            y = _tree_sum(ys).astype(BF).astype(F32)
            rs = jax.nn.sigmoid(rmax[:, 0:1]).astype(BF).astype(F32)
            y = (y * rs).astype(BF).astype(F32)
            sel = lax.broadcasted_iota(jnp.int32, (16, 1), 0) == (idx - base)
            hb = jnp.where(sel, h2f + y, h2f)
            og = (x1g + mod_row(5) * hb).astype(BF)
            for t in range(NT):
                wait(cp_out(t))
            out_v[pl.ds(base, 16), :] = og
            fin = mk(out_v.at[pl.ds(base, 16)], out_hbm.at[pl.ds(base, 16)], sem_out.at[0])
            fin.start()
            fin.wait()

    return kernel


def build(vmem_mb=110, scopes=False, **opts):

    @jax.jit
    def fn(A_x, A_k_cache, A_v_cache, A_wq, A_wo, B_x, B_w_r, B_w_gate, B_w_up, B_w_down, c, w_mod):
        x = A_x.reshape(S, D)
        k = A_k_cache.reshape(HKV, SK, DH)
        v = A_v_cache.reshape(HKV, SK, DH)
        any_spec = pl.BlockSpec(memory_space=pl.ANY)
        vm = pl.BlockSpec(memory_space=pltpu.VMEM)
        out = pl.pallas_call(
            _make_kernel(scopes, opts),
            out_shape=jax.ShapeDtypeStruct((S, D), BF),
            in_specs=[vm, vm] + [any_spec] * 9,
            out_specs=any_spec,
            scratch_shapes=[
                pltpu.VMEM((S, D), BF),
                pltpu.VMEM((HKV, W, DH), BF),
                pltpu.VMEM((HKV, W, DH), BF),
                pltpu.VMEM((HKV, W // 128, DH, 128), BF),
                pltpu.VMEM((D, HQ * DH), BF),
                pltpu.VMEM((HQ * DH, D), BF),
                pltpu.VMEM((D, F), BF),
                pltpu.VMEM((D, F), BF),
                pltpu.VMEM((F, D), BF),
                pltpu.VMEM((D, 4 * D), BF),
                pltpu.VMEM((S, D), BF),
                pltpu.VMEM((S, D), F32),
                pltpu.VMEM((S, D), BF),
                pltpu.VMEM((S, 128), F32),
                pltpu.VMEM((2, REP, TQ, DH), BF),
                pltpu.VMEM((2, REP, TQ, DH), BF),
                pltpu.VMEM((16, 6 * D), F32),
                pltpu.VMEM((8, 128), U32),
                pltpu.VMEM((1, D), F32),
                pltpu.SemaphoreType.DMA((5,)),
                pltpu.SemaphoreType.DMA((5,)),
                pltpu.SemaphoreType.DMA((5,)),
                pltpu.SemaphoreType.DMA((2,)),
                pltpu.SemaphoreType.DMA((1,)),
            ],
            compiler_params=pltpu.CompilerParams(vmem_limit_bytes=vmem_mb * 1024 * 1024),
        )(c, B_w_r, x, k, v, A_wq, A_wo, B_w_gate, B_w_up, B_w_down, w_mod)
        return out.reshape(1, S, D)

    return fn


_IMPL = build()


@jax.jit
def pallas_adaLN_cond__sliding_block_cached__moe_arch_mod__prompt_kernel(
    A_x: jax.Array,
    A_k_cache: jax.Array,
    A_v_cache: jax.Array,
    A_wq: jax.Array,
    A_wo: jax.Array,
    B_x: jax.Array,
    B_w_r: jax.Array,
    B_w_gate: jax.Array,
    B_w_up: jax.Array,
    B_w_down: jax.Array,
    c: jax.Array,
    w_mod: jax.Array,
):
    return _IMPL(A_x, A_k_cache, A_v_cache, A_wq, A_wo, B_x, B_w_r, B_w_gate, B_w_up, B_w_down, c, w_mod)
```

```python
import contextlib

import jax
import jax.numpy as jnp
from jax import lax
import jax.experimental.pallas as pl
import jax.experimental.pallas.tpu as pltpu

S, D, HQ, HKV, DH, SK, F = 2048, 1024, 32, 4, 128, 2048, 3584
W = min(4096, max(256, SK // 4))
REP = HQ // HKV
GW = REP * DH
NP = D // 128
TQ = 128
NT = S // TQ
NS = NT * HKV
CH = TQ // REP
EPS = 1e-5
BF = jnp.bfloat16
F32 = jnp.float32
U32 = jnp.uint32
LOG2E = 1.4426950408889634
QSCALE = DH ** -0.5 * LOG2E


def _ln(xf, rel=None):
    m = jnp.sum(xf, axis=-1, keepdims=True)
    if rel is not None:
        m = m + rel
    m = m * (1.0 / D)
    d = xf - m
    v = jnp.sum(d * d, axis=-1, keepdims=True) * (1.0 / D)
    return d * lax.rsqrt(v + EPS)


def _recip(l):
    r = pl.reciprocal(l, approx=True)
    return r * (2.0 - l * r)


def _tree_sum(xs):
    while len(xs) > 1:
        xs = [xs[i] + xs[i + 1] if i + 1 < len(xs) else xs[i] for i in range(0, len(xs), 2)]
    return xs[0]


def _make_kernel(scopes, opts):
    NTMM = opts.get("nt", False)
    POST_DL = opts.get("pdl", 1)
    VMOD = opts.get("vmod", True)
    AMAX = opts.get("amax", True)

    def scope(name):
        return jax.named_scope(name) if scopes else contextlib.nullcontext()

    def kernel(c_ref, wr_ref, x_hbm, k_hbm, v_hbm, wq_hbm, wo_hbm, wg_hbm, wu_hbm, wd_hbm, wm_hbm,
               out_hbm,
               x_v, k_v, v_v, kt_v, wq_v, wo_v, wg_v, wu_v, wd_v, wm_v, out_v, acc_v, h_v, r_v,
               q_s, o_s, mod_v, zero_s, wr_s, csb_v,
               sem_x, sem_wm, sem_g0, sem_rest, sem_out):
        mk = pltpu.make_async_copy

        def cp_x(t0, n, s):
            return [mk(x_hbm.at[pl.ds(t0 * TQ, n * TQ)], x_v.at[pl.ds(t0 * TQ, n * TQ), pl.ds(0, D)], sem_x.at[s])]

        def cp_wm(c0, n, s):
            return [mk(wm_hbm.at[:, pl.ds(c0, n)], wm_v.at[:, pl.ds(c0 % (4 * D), n)], sem_wm.at[s])]

        def cp_wq0(half):
            c0 = half * (GW // 2)
            return [mk(wq_hbm.at[:, pl.ds(c0, GW // 2)], wq_v.at[:, pl.ds(c0, GW // 2)], sem_g0.at[half])]

        def cp_kv0():
            return [mk(k_hbm.at[0, pl.ds(SK - W, W), :], k_v.at[0], sem_g0.at[2]),
                    mk(v_hbm.at[0, pl.ds(SK - W, W), :], v_v.at[0], sem_g0.at[3])]

        def cp_wo0():
            return [mk(wo_hbm.at[pl.ds(0, GW)], wo_v.at[pl.ds(0, GW), pl.ds(0, D)], sem_g0.at[4])]

        def cp_rest():
            n = HKV - 1
            return [mk(wq_hbm.at[:, pl.ds(GW, n * GW)], wq_v.at[:, pl.ds(GW, n * GW)], sem_rest.at[0]),
                    mk(wo_hbm.at[pl.ds(GW, n * GW)], wo_v.at[pl.ds(GW, n * GW), pl.ds(0, D)], sem_rest.at[0]),
                    mk(k_hbm.at[pl.ds(1, n), pl.ds(SK - W, W), :], k_v.at[pl.ds(1, n)], sem_rest.at[0]),
                    mk(v_hbm.at[pl.ds(1, n), pl.ds(SK - W, W), :], v_v.at[pl.ds(1, n)], sem_rest.at[0])]

        def cp_wm_b():
            return cp_wm(2 * D, 2 * D, 4) + cp_wm(4 * D, 2 * D, 4)

        def cp_ff():
            return [mk(wg_hbm, wg_v.at[:, pl.ds(0, F)], sem_rest.at[1]), mk(wu_hbm, wu_v.at[:, pl.ds(0, F)], sem_rest.at[1]), mk(wd_hbm, wd_v.at[:, pl.ds(0, D)], sem_rest.at[1])]

        def cp_out(t):
            r0 = t * TQ if isinstance(t, int) else pl.multiple_of(t * TQ, TQ)
            return [mk(out_v.at[pl.ds(r0, TQ), pl.ds(0, D)], out_hbm.at[pl.ds(r0, TQ)], sem_out.at[0])]

        def start(cps):
            for cp in cps:
                cp.start()

        def wait(cps):
            for cp in cps:
                cp.wait()

        def rows(r0, n):
            return pl.ds(r0 if isinstance(r0, int) else pl.multiple_of(r0, n), n)

        state = {"dead": [], "rel": None}

        def tok(v):
            u = pltpu.bitcast(v[0:16, 0:128] if v.dtype == BF else v[0:8, 0:128], U32)
            return u & zero_s[...]

        def take_rel():
            if state["rel"] is None:
                return None
            return jnp.concatenate([pltpu.bitcast(state["rel"], F32)[:, 0:1]] * (CH // 8), axis=0)

        def with_dead(lhs):
            ready = [z for (z, n) in state["dead"] if n <= 0]
            state["dead"] = [(z, n - 1) for (z, n) in state["dead"] if n > 0]
            if not ready:
                return lhs
            z = ready[0]
            for z2 in ready[1:]:
                z = z | z2
            n = lhs.shape[0]
            last = pltpu.bitcast(pltpu.bitcast(lhs[n - 16:n, :], U32) | z, BF)
            return jnp.concatenate([lhs[0:n - 16, :], last], axis=0)

        def reset_tokens():
            state["dead"] = []
            state["rel"] = None

        def cs_dot(cs16, c0, n):
            ps = [jnp.dot(cs16[:, k * 128:(k + 1) * 128], wm_v[k * 128:(k + 1) * 128, c0:c0 + n],
                          preferred_element_type=F32) for k in range(NP)]
            return _tree_sum(ps).astype(BF).astype(F32)

        def mod_row(which):
            return mod_v[0:1, which * D:(which + 1) * D]

        def one_plus(which):
            return (1 + mod_row(which).astype(BF)).astype(F32)

        def pre_chunk(t, ci):
            sl = rows(t * TQ + ci * CH, CH)
            h = (_ln(x_v[sl, 0:D].astype(F32), take_rel()) * one_plus(1) + mod_row(0)).astype(BF)
            h_v[sl, 0:D] = h
            state["dead"].append((tok(h[CH - 16:CH, D - 128:D]), 0))

        def ln2(x1, rel=None):
            return _ln(x1, rel) * one_plus(4) + mod_row(3)

        def post_chunk(t, ci):
            sl = rows(t * TQ + ci * CH, CH)
            x1 = acc_v[sl, 0:D]
            h2 = ln2(x1, take_rel())
            r = jnp.sum(h2 * wr_s[...], axis=-1, keepdims=True).astype(BF).astype(F32)
            ob = (x1 + mod_row(5) * h2).astype(BF)
            out_v[sl, 0:D] = ob
            r_v[sl, :] = jnp.broadcast_to(r, (CH, 128))
            state["dead"].append((tok(ob[CH - 16:CH, D - 128:D]) | tok(jnp.broadcast_to(r[CH - 8:CH, :], (8, 128))), POST_DL))

        def mod_chunk(p, ci, acc):
            c0 = pl.multiple_of(p * 128, 128)
            ks = slice(ci * 128, (ci + 1) * 128)
            prod = wm_v[ks, pl.ds(c0, 128)].astype(F32) * csb_v[ks, :]
            part = _tree_sum([prod[i * 8:(i + 1) * 8, :] for i in range(16)])
            acc = part if acc is None else acc + part
            if ci == REP - 1:
                tot = jnp.sum(acc, axis=0, keepdims=True).astype(BF).astype(F32)
                dst = pl.multiple_of(jnp.where(c0 >= 2 * D, c0, c0 + 4 * D), 128)
                mod_v[0:8, pl.ds(dst, 128)] = jnp.broadcast_to(tot, (8, 128))
            state["dead"].append((tok(acc), 0))
            return acc

        def q_item(gq, tq, n, slot):
            c0 = gq * GW + n * DH
            if not isinstance(c0, int):
                c0 = pl.multiple_of(c0, DH)
            q = jnp.dot(h_v[rows(tq * TQ, TQ), 0:D], wq_v[:, pl.ds(c0, DH)], preferred_element_type=F32)
            q_s[slot, n] = (q * QSCALE).astype(BF)

        def o_item(go, to, n, slot, fin):
            oo = jnp.concatenate([o_s[slot, k] for k in range(REP)], axis=1)
            cs_ = slice(n * 128, (n + 1) * 128)
            part = jnp.dot(oo, wo_v[rows(go * GW, GW), cs_], preferred_element_type=F32)
            sl = rows(to * TQ, TQ)
            if fin:
                ga = mod_v[0:1, 2 * D + n * 128:2 * D + (n + 1) * 128]
                acc_v[sl, cs_] = x_v[sl, cs_].astype(F32) + ga * (acc_v[sl, cs_] + part)
            else:
                acc_v[sl, cs_] += part

        def s_item(g, hh, slot):
            qq = with_dead(q_s[slot, hh])
            if NTMM:
                return lax.dot_general(qq, k_v[g], (((1,), (1,)), ((), ())), preferred_element_type=F32)
            return jnp.concatenate([jnp.dot(qq, kt_v[g, n], preferred_element_type=F32)
                                    for n in range(W // 128)], axis=1)

        def softmax_item(s):
            m = jnp.max(s, axis=-1, keepdims=True)
            p = jnp.exp2(s - m)
            l = jnp.sum(p, axis=-1, keepdims=True)
            return p.astype(BF), _recip(l)

        def pv_item(g, hh, slot, p, rl):
            o = jnp.dot(p, v_v[g], preferred_element_type=F32)
            state["rel"] = tok(o)
            o_s[slot, hh] = (o * rl).astype(BF)

        def step(j, slot, do_q=True, do_o=True, fin=False, pre_t=None, post_t=None, mod_p=None, amax=None):
            g = j // NT
            gq, tq = (j + 1) // NT, (j + 1) % NT
            go, to = (j - 1) // NT, (j - 1) % NT
            s_next = s_item(g, 0, slot)
            macc = None
            for hh in range(REP):
                s_cur = s_next
                if hh + 1 < REP:
                    s_next = s_item(g, hh + 1, slot)
                if do_q:
                    q_item(gq, tq, hh, 1 - slot)
                if pre_t is not None:
                    pre_chunk(pre_t, hh)
                if post_t is not None:
                    post_chunk(post_t, hh)
                if mod_p is not None:
                    macc = mod_chunk(mod_p, hh, macc)
                if amax is not None:
                    n_ = amax[0] // REP
                    amax[1].append(best_rows(hh * n_, n_))
                    state["dead"].append((tok(amax[1][-1][0]) | tok(pltpu.bitcast(amax[1][-1][1], F32)), 0))
                p, rl = softmax_item(s_cur)
                if do_o:
                    o_item(go, to, hh, 1 - slot, fin)
                pv_item(g, hh, slot, p, rl)

        def transpose_k(g):
            if not NTMM:
                for n in range(W // 128):
                    kt_v[g, n] = k_v[g, n * 128:(n + 1) * 128, :].astype(F32).T.astype(BF)

        def combine_best(items):
            while len(items) > 1:
                nxt = []
                for i in range(0, len(items) - 1, 2):
                    (av, ai), (bv, bi) = items[i], items[i + 1]
                    upd = bv > av
                    nxt.append((jnp.where(upd, bv, av), jnp.where(upd, bi, ai)))
                if len(items) % 2:
                    nxt.append(items[-1])
                items = nxt
            return items[0]

        def best_rows(r0, n):
            sub = lax.broadcasted_iota(jnp.int32, (8, 128), 0)
            return combine_best([(r_v[r0 + i * 8:r0 + (i + 1) * 8, :], sub + (r0 + i * 8)) for i in range(n // 8)])

        with scope("prologue"):
            start(cp_x(0, 1, 0))
            for ci in range(4):
                start(cp_wm(ci * 512, 512, ci))
            cs = c_ref[...].astype(F32)
            cs16 = jnp.broadcast_to((cs * jax.nn.sigmoid(cs)).astype(BF), (16, D))
            zero_s[...] = jnp.zeros((8, 128), U32)
            wr_s[...] = wr_ref[...].astype(F32).reshape(1, D)
            if VMOD:
                csb_v[...] = jnp.broadcast_to(cs16[0:1, :].astype(F32), (128, D)).T

            def zero_body(i, carry):
                acc_v[pl.ds(pl.multiple_of(i * 128, 128), 128), 0:D] = jnp.zeros((128, D), F32)
                return carry
            lax.fori_loop(0, S // 128, zero_body, 0)
            wait(cp_x(0, 1, 0))
            start(cp_wq0(0))
            start(cp_wq0(1))
            start(cp_x(1, 1, 1))
            start(cp_kv0())
            start(cp_x(2, 1, 2))
            for ci in range(4):
                wait(cp_wm(ci * 512, 512, ci))
                mod_v[:, ci * 512:(ci + 1) * 512] = cs_dot(cs16, ci * 512, 512)
            reset_tokens()
            for ci in range(REP):
                pre_chunk(0, ci)
            reset_tokens()
            wait(cp_wq0(0))
            start(cp_x(3, 2, 3))
            start(cp_wo0())
            for n in range(REP // 2):
                q_item(0, 0, n, 0)
            wait(cp_wq0(1))
            start(cp_x(5, NT - 5, 4))
            for n in range(REP // 2, REP):
                q_item(0, 0, n, 0)
            wait(cp_x(1, 1, 1))
            for ci in range(REP):
                pre_chunk(1, ci)
            wait(cp_kv0())
            transpose_k(0)
            wait(cp_x(2, 1, 2))

        with scope("first"):
            reset_tokens()
            step(0, 0, do_o=False, pre_t=2)
            wait(cp_wo0())
            wait(cp_x(3, 2, 3))
            start(cp_rest())
            if opts.get("ffat", 0) == 0:
                start(cp_wm_b())
                start(cp_ff())
            elif opts.get("ffat", 0) == 1:
                start(cp_wm_b())

        def body_a0(i, carry):
            j = 2 * i + 1

            @pl.when(i == 1)
            def _():
                wait(cp_x(5, NT - 5, 4))

            reset_tokens()
            with scope("A0"):
                step(j, 1, pre_t=j + 2)
                step(j + 1, 0, pre_t=jnp.minimum(j + 3, NT - 1))
            return carry

        lax.fori_loop(0, NT // 2 - 1, body_a0, 0)

        with scope("mid"):
            wait(cp_rest())
            if opts.get("ffat", 0) == 2:
                start(cp_wm_b())
            if opts.get("ffat", 0) >= 1:
                start(cp_ff())
            if VMOD:
                wait(cp_wm_b())
            for g in range(1, HKV):
                transpose_k(g)

        def body_a1(i, carry):
            j = 2 * i + 1
            reset_tokens()
            with scope("A1"):
                j0 = NT - 1
                mp = (lambda jj: jnp.minimum(jj - j0, 4 * NP - 1)) if VMOD else (lambda jj: None)
                step(j, 1, mod_p=mp(j))
                step(j + 1, 0, mod_p=mp(j + 1))
            return carry

        JB = (HKV - 1) * NT + 1
        lax.fori_loop(NT // 2 - 1, (JB - 1) // 2, body_a1, 0)

        with scope("modb"):
            if not VMOD:
                wait(cp_wm_b())
                mod_v[:, 2 * D:4 * D] = cs_dot(cs16, 2 * D, 2 * D)
                mod_v[:, 4 * D:6 * D] = cs_dot(cs16, 0, 2 * D)

        def body_b(i, carry):
            j = 2 * i + 1
            t = j - JB - 1
            reset_tokens()
            with scope("B"):
                step(j, 1, fin=True, post_t=jnp.maximum(t, 0))
                step(j + 1, 0, fin=True, post_t=t + 1)

                @pl.when(t >= 0)
                def _():
                    start(cp_out(t))
                start(cp_out(t + 1))
            return carry

        lax.fori_loop((JB - 1) // 2, (NS - 2) // 2, body_b, 0)

        with scope("last"):
            reset_tokens()
            parts = []
            step(NS - 1, 1, do_q=False, fin=True, post_t=NT - 3, amax=((NT - 3) * TQ, parts) if AMAX else None)
            start(cp_out(NT - 3))
            for n in range(NP):
                reset_tokens()
                o_item(HKV - 1, NT - 1, n, 1, True)
                post_chunk(NT - 2, n)
            start(cp_out(NT - 2))
            if AMAX:
                parts.append(best_rows((NT - 3) * TQ, 2 * TQ))
                av, ai = combine_best(parts)
            else:
                av, ai = best_rows(0, (NT - 1) * TQ)
            reset_tokens()
            for ci in range(REP):
                post_chunk(NT - 1, ci)
            start(cp_out(NT - 1))
            bv, bi = best_rows((NT - 1) * TQ, TQ)
            upd = bv > av
            bv, bi = jnp.where(upd, bv, av), jnp.where(upd, bi, ai)

        with scope("tail"):
            rmax = jnp.max(bv, axis=0, keepdims=True)
            idx = jnp.minimum(jnp.min(jnp.where(bv == rmax, bi, S)), S - 1)
            base = pl.multiple_of((idx // 16) * 16, 16)
            x1g = acc_v[pl.ds(base, 16), 0:D]
            h2f = ln2(x1g)
            h2g = h2f.astype(BF)
            wait(cp_ff())
            acts = []
            for n in range(F // 128):
                fs = slice(n * 128, (n + 1) * 128)
                gt = jnp.dot(h2g, wg_v[:, fs], preferred_element_type=F32).astype(BF).astype(F32)
                up = jnp.dot(h2g, wu_v[:, fs], preferred_element_type=F32).astype(BF).astype(F32)
                acts.append(((gt * jax.nn.sigmoid(gt)).astype(BF).astype(F32) * up).astype(BF))
            ys = [jnp.dot(acts[n], wd_v[n * 128:(n + 1) * 128, 0:D], preferred_element_type=F32)
                  for n in range(F // 128)]
            y = _tree_sum(ys).astype(BF).astype(F32)
            rs = jax.nn.sigmoid(rmax[:, 0:1]).astype(BF).astype(F32)
            y = (y * rs).astype(BF).astype(F32)
            sel = lax.broadcasted_iota(jnp.int32, (16, 1), 0) == (idx - base)
            hb = jnp.where(sel, h2f + y, h2f)
            og = (x1g + mod_row(5) * hb).astype(BF)
            for t in range(NT):
                wait(cp_out(t))
            out_v[pl.ds(base, 16), 0:D] = og
            fin = mk(out_v.at[pl.ds(base, 16), pl.ds(0, D)], out_hbm.at[pl.ds(base, 16)], sem_out.at[0])
            fin.start()
            fin.wait()

    return kernel


def build(vmem_mb=110, scopes=False, **opts):

    @jax.jit
    def fn(A_x, A_k_cache, A_v_cache, A_wq, A_wo, B_x, B_w_r, B_w_gate, B_w_up, B_w_down, c, w_mod):
        x = A_x.reshape(S, D)
        k = A_k_cache.reshape(HKV, SK, DH)
        v = A_v_cache.reshape(HKV, SK, DH)
        def P(shape, dtype, letter):
            n = opts.get("pads", {}).get(letter, 0)
            return pltpu.VMEM((shape[0], shape[1] + 128 * n), dtype)

        any_spec = pl.BlockSpec(memory_space=pl.ANY)
        vm = pl.BlockSpec(memory_space=pltpu.VMEM)
        out = pl.pallas_call(
            _make_kernel(scopes, opts),
            out_shape=jax.ShapeDtypeStruct((S, D), BF),
            in_specs=[vm, vm] + [any_spec] * 9,
            out_specs=any_spec,
            scratch_shapes=[
                P((S, D), BF, "x"),
                pltpu.VMEM((HKV, W, DH), BF),
                pltpu.VMEM((HKV, W, DH), BF),
                pltpu.VMEM((HKV, W // 128, DH, 128), BF),
                P((D, HQ * DH), BF, "q"),
                P((HQ * DH, D), BF, "o"),
                P((D, F), BF, "f"),
                P((D, F), BF, "f"),
                P((F, D), BF, "f"),
                P((D, 4 * D), BF, "m"),
                P((S, D), BF, "x"),
                P((S, D), F32, "a"),
                P((S, D), BF, "h"),
                pltpu.VMEM((S, 128), F32),
                pltpu.VMEM((2, REP, TQ, DH), BF),
                pltpu.VMEM((2, REP, TQ, DH), BF),
                pltpu.VMEM((16, 6 * D), F32),
                pltpu.VMEM((8, 128), U32),
                pltpu.VMEM((1, D), F32),
                pltpu.VMEM((D, 128), F32),
                pltpu.SemaphoreType.DMA((5,)),
                pltpu.SemaphoreType.DMA((5,)),
                pltpu.SemaphoreType.DMA((5,)),
                pltpu.SemaphoreType.DMA((2,)),
                pltpu.SemaphoreType.DMA((1,)),
            ],
            compiler_params=pltpu.CompilerParams(vmem_limit_bytes=vmem_mb * 1024 * 1024),
        )(c, B_w_r, x, k, v, A_wq, A_wo, B_w_gate, B_w_up, B_w_down, w_mod)
        return out.reshape(1, S, D)

    return fn


_IMPL = build(pads={'o': 1})


@jax.jit
def pallas_adaLN_cond__sliding_block_cached__moe_arch_mod__prompt_kernel(
    A_x: jax.Array,
    A_k_cache: jax.Array,
    A_v_cache: jax.Array,
    A_wq: jax.Array,
    A_wo: jax.Array,
    B_x: jax.Array,
    B_w_r: jax.Array,
    B_w_gate: jax.Array,
    B_w_up: jax.Array,
    B_w_down: jax.Array,
    c: jax.Array,
    w_mod: jax.Array,
):
    return _IMPL(A_x, A_k_cache, A_v_cache, A_wq, A_wo, B_x, B_w_r, B_w_gate, B_w_up, B_w_down, c, w_mod)
```

```python
import jax
import jax.numpy as jnp
from jax import lax
import jax.experimental.pallas as pl
import jax.experimental.pallas.tpu as pltpu

S, D, HQ, HKV, DH, SK, F = 2048, 1024, 32, 4, 128, 2048, 3584
W = min(4096, max(256, SK // 4))
REP = HQ // HKV
GW = REP * DH
NP = D // 128
TQ = 128
NT = S // TQ
NS = NT * HKV
CH = TQ // REP
EPS = 1e-5
BF = jnp.bfloat16
F32 = jnp.float32
U32 = jnp.uint32
LOG2E = 1.4426950408889634
QSCALE = DH ** -0.5 * LOG2E


def _ln(xf, rel=None):
    m = jnp.sum(xf, axis=-1, keepdims=True)
    if rel is not None:
        m = m + rel
    m = m * (1.0 / D)
    d = xf - m
    v = jnp.sum(d * d, axis=-1, keepdims=True) * (1.0 / D)
    return d * lax.rsqrt(v + EPS)


def _recip(l):
    r = pl.reciprocal(l, approx=True)
    return r * (2.0 - l * r)


def _tree_sum(xs):
    while len(xs) > 1:
        xs = [xs[i] + xs[i + 1] if i + 1 < len(xs) else xs[i] for i in range(0, len(xs), 2)]
    return xs[0]


def _make_kernel():
    def kernel(c_ref, wr_ref, x_hbm, k_hbm, v_hbm, wq_hbm, wo_hbm, wg_hbm, wu_hbm, wd_hbm, wm_hbm,
               out_hbm,
               x_v, k_v, v_v, kt_v, wq_v, wo_v, wg_v, wu_v, wd_v, wm_v, out_v, acc_v, h_v, r_v,
               q_s, o_s, mod_v, zero_s, wr_s, csb_v, c_v, wrb_v,
               sem_x, sem_wm, sem_g0, sem_rest, sem_out):
        mk = pltpu.make_async_copy

        def cp_x(t0, n, s):
            return [mk(x_hbm.at[pl.ds(t0 * TQ, n * TQ)], x_v.at[pl.ds(t0 * TQ, n * TQ), pl.ds(0, D)], sem_x.at[s])]

        def cp_wm(c0, n, s):
            return [mk(wm_hbm.at[:, pl.ds(c0, n)], wm_v.at[:, pl.ds(c0 % (4 * D), n)], sem_wm.at[s])]

        def cp_wq0(half):
            c0 = half * (GW // 2)
            return [mk(wq_hbm.at[:, pl.ds(c0, GW // 2)], wq_v.at[:, pl.ds(c0, GW // 2)], sem_g0.at[half])]

        def cp_kv0():
            return [mk(k_hbm.at[0, pl.ds(SK - W, W), :], k_v.at[0], sem_g0.at[2]),
                    mk(v_hbm.at[0, pl.ds(SK - W, W), :], v_v.at[0], sem_g0.at[3])]

        def cp_wo0():
            return [mk(wo_hbm.at[pl.ds(0, GW)], wo_v.at[pl.ds(0, GW), pl.ds(0, D)], sem_g0.at[4])]

        def cp_rest():
            n = HKV - 1
            return [mk(wq_hbm.at[:, pl.ds(GW, n * GW)], wq_v.at[:, pl.ds(GW, n * GW)], sem_rest.at[0]),
                    mk(wo_hbm.at[pl.ds(GW, n * GW)], wo_v.at[pl.ds(GW, n * GW), pl.ds(0, D)], sem_rest.at[0]),
                    mk(k_hbm.at[pl.ds(1, n), pl.ds(SK - W, W), :], k_v.at[pl.ds(1, n)], sem_rest.at[0]),
                    mk(v_hbm.at[pl.ds(1, n), pl.ds(SK - W, W), :], v_v.at[pl.ds(1, n)], sem_rest.at[0])]

        def cp_wm_b():
            return cp_wm(2 * D, 2 * D, 4) + cp_wm(4 * D, 2 * D, 4)

        def cp_ff():
            return [mk(wg_hbm, wg_v.at[:, pl.ds(0, F)], sem_rest.at[1]), mk(wu_hbm, wu_v.at[:, pl.ds(0, F)], sem_rest.at[1]), mk(wd_hbm, wd_v.at[:, pl.ds(0, D)], sem_rest.at[1])]

        def cp_out(t):
            r0 = t * TQ if isinstance(t, int) else pl.multiple_of(t * TQ, TQ)
            return [mk(out_v.at[pl.ds(r0, TQ), pl.ds(0, D)], out_hbm.at[pl.ds(r0, TQ)], sem_out.at[0])]

        def start(cps):
            for cp in cps:
                cp.start()

        def wait(cps):
            for cp in cps:
                cp.wait()

        def rows(r0, n):
            return pl.ds(r0 if isinstance(r0, int) else pl.multiple_of(r0, n), n)

        state = {"dead": [], "rel": None}

        def tok(v):
            u = pltpu.bitcast(v[0:16, 0:128] if v.dtype == BF else v[0:8, 0:128], U32)
            return u & zero_s[...]

        def take_rel():
            if state["rel"] is None:
                return None
            return jnp.concatenate([pltpu.bitcast(state["rel"], F32)[:, 0:1]] * (CH // 8), axis=0)

        def with_dead(lhs):
            ready = [z for (z, n) in state["dead"] if n <= 0]
            state["dead"] = [(z, n - 1) for (z, n) in state["dead"] if n > 0]
            if not ready:
                return lhs
            z = ready[0]
            for z2 in ready[1:]:
                z = z | z2
            n = lhs.shape[0]
            last = pltpu.bitcast(pltpu.bitcast(lhs[n - 16:n, :], U32) | z, BF)
            return jnp.concatenate([lhs[0:n - 16, :], last], axis=0)

        def reset_tokens():
            state["dead"] = []
            state["rel"] = None

        def cs_dot(cs16, c0, n):
            ps = [jnp.dot(cs16[:, k * 128:(k + 1) * 128], wm_v[k * 128:(k + 1) * 128, c0:c0 + n],
                          preferred_element_type=F32) for k in range(NP)]
            return _tree_sum(ps).astype(BF).astype(F32)

        def mod_row(which):
            return mod_v[0:1, which * D:(which + 1) * D]

        def one_plus(which):
            return (1 + mod_row(which).astype(BF)).astype(F32)

        def pre_chunk(t, ci):
            sl = rows(t * TQ + ci * CH, CH)
            h = (_ln(x_v[sl, 0:D].astype(F32), take_rel()) * one_plus(1) + mod_row(0)).astype(BF)
            h_v[sl, 0:D] = h
            state["dead"].append((tok(h[CH - 16:CH, D - 128:D]), 0))

        def ln2(x1, rel=None):
            return _ln(x1, rel) * one_plus(4) + mod_row(3)

        def post_chunk(t, ci):
            sl = rows(t * TQ + ci * CH, CH)
            x1 = acc_v[sl, 0:D]
            h2 = ln2(x1, take_rel())
            r = jnp.sum(h2 * wr_s[...], axis=-1, keepdims=True).astype(BF).astype(F32)
            ob = (x1 + mod_row(5) * h2).astype(BF)
            out_v[sl, 0:D] = ob
            r_v[sl, :] = jnp.broadcast_to(r, (CH, 128))
            state["dead"].append((tok(ob[CH - 16:CH, D - 128:D]) | tok(jnp.broadcast_to(r[CH - 8:CH, :], (8, 128))), 1))

        def mod_chunk(p, ci, acc):
            c0 = pl.multiple_of(p * 128, 128)
            ks = slice(ci * 128, (ci + 1) * 128)
            prod = wm_v[ks, pl.ds(c0, 128)].astype(F32) * csb_v[ks, :]
            part = _tree_sum([prod[i * 8:(i + 1) * 8, :] for i in range(16)])
            acc = part if acc is None else acc + part
            if ci == REP - 1:
                tot = jnp.sum(acc, axis=0, keepdims=True).astype(BF).astype(F32)
                dst = pl.multiple_of(jnp.where(c0 >= 2 * D, c0, c0 + 4 * D), 128)
                mod_v[0:8, pl.ds(dst, 128)] = jnp.broadcast_to(tot, (8, 128))
            state["dead"].append((tok(acc), 0))
            return acc

        def q_item(gq, tq, n, slot):
            c0 = gq * GW + n * DH
            if not isinstance(c0, int):
                c0 = pl.multiple_of(c0, DH)
            q = jnp.dot(h_v[rows(tq * TQ, TQ), 0:D], wq_v[:, pl.ds(c0, DH)], preferred_element_type=F32)
            q_s[slot, n] = (q * QSCALE).astype(BF)

        def o_item(go, to, n, slot, fin):
            oo = jnp.concatenate([o_s[slot, k] for k in range(REP)], axis=1)
            cs_ = slice(n * 128, (n + 1) * 128)
            part = jnp.dot(oo, wo_v[rows(go * GW, GW), cs_], preferred_element_type=F32)
            sl = rows(to * TQ, TQ)
            if fin:
                ga = mod_v[0:1, 2 * D + n * 128:2 * D + (n + 1) * 128]
                acc_v[sl, cs_] = x_v[sl, cs_].astype(F32) + ga * (acc_v[sl, cs_] + part)
            else:
                acc_v[sl, cs_] += part

        def s_item(g, hh, slot):
            qq = with_dead(q_s[slot, hh])
            return jnp.concatenate([jnp.dot(qq, kt_v[g, n], preferred_element_type=F32)
                                    for n in range(W // 128)], axis=1)

        def softmax_item(s):
            m = jnp.max(s, axis=-1, keepdims=True)
            p = jnp.exp2(s - m)
            l = jnp.sum(p, axis=-1, keepdims=True)
            return p.astype(BF), _recip(l)

        def pv_item(g, hh, slot, p, rl):
            o = jnp.dot(p, v_v[g], preferred_element_type=F32)
            state["rel"] = tok(o)
            o_s[slot, hh] = (o * rl).astype(BF)

        def step(j, slot, do_q=True, do_o=True, fin=False, pre_t=None, post_t=None, mod_p=None, amax=None):
            g = j // NT
            gq, tq = (j + 1) // NT, (j + 1) % NT
            go, to = (j - 1) // NT, (j - 1) % NT
            s_next = s_item(g, 0, slot)
            macc = None
            for hh in range(REP):
                s_cur = s_next
                if hh + 1 < REP:
                    s_next = s_item(g, hh + 1, slot)
                if do_q:
                    q_item(gq, tq, hh, 1 - slot)
                if pre_t is not None:
                    pre_chunk(pre_t, hh)
                if post_t is not None:
                    post_chunk(post_t, hh)
                if mod_p is not None:
                    macc = mod_chunk(mod_p, hh, macc)
                if amax is not None:
                    n_ = amax[0] // REP
                    amax[1].append(best_rows(hh * n_, n_))
                    state["dead"].append((tok(amax[1][-1][0]) | tok(pltpu.bitcast(amax[1][-1][1], F32)), 0))
                p, rl = softmax_item(s_cur)
                if do_o:
                    o_item(go, to, hh, 1 - slot, fin)
                pv_item(g, hh, slot, p, rl)

        def transpose_k(g):
            for n in range(W // 128):
                kt_v[g, n] = k_v[g, n * 128:(n + 1) * 128, :].astype(F32).T.astype(BF)

        def combine_best(items):
            while len(items) > 1:
                nxt = []
                for i in range(0, len(items) - 1, 2):
                    (av, ai), (bv, bi) = items[i], items[i + 1]
                    upd = bv > av
                    nxt.append((jnp.where(upd, bv, av), jnp.where(upd, bi, ai)))
                if len(items) % 2:
                    nxt.append(items[-1])
                items = nxt
            return items[0]

        def best_rows(r0, n):
            sub = lax.broadcasted_iota(jnp.int32, (8, 128), 0)
            return combine_best([(r_v[r0 + i * 8:r0 + (i + 1) * 8, :], sub + (r0 + i * 8)) for i in range(n // 8)])

        cp_small = [mk(c_ref, c_v, sem_rest.at[2]), mk(wr_ref, wrb_v, sem_rest.at[2])]
        start(cp_small)
        start(cp_x(0, 1, 0))
        for ci in range(4):
            start(cp_wm(ci * 512, 512, ci))
        zero_s[...] = jnp.zeros((8, 128), U32)

        def zero_body(i, carry):
            acc_v[pl.ds(pl.multiple_of(i * 128, 128), 128), 0:D] = jnp.zeros((128, D), F32)
            return carry
        lax.fori_loop(0, S // 128, zero_body, 0)
        wait(cp_small)
        cs = c_v[...].astype(F32)
        cs16 = jnp.broadcast_to((cs * jax.nn.sigmoid(cs)).astype(BF), (16, D))
        wr_s[...] = wrb_v[...].astype(F32).reshape(1, D)
        csb_v[...] = jnp.broadcast_to(cs16[0:1, :].astype(F32), (128, D)).T
        wait(cp_x(0, 1, 0))
        start(cp_wq0(0))
        start(cp_wq0(1))
        start(cp_x(1, 1, 1))
        start(cp_kv0())
        start(cp_x(2, 1, 2))
        for ci in range(4):
            wait(cp_wm(ci * 512, 512, ci))
            mod_v[:, ci * 512:(ci + 1) * 512] = cs_dot(cs16, ci * 512, 512)
        reset_tokens()
        for ci in range(REP):
            pre_chunk(0, ci)
        reset_tokens()
        wait(cp_wq0(0))
        start(cp_x(3, 2, 3))
        start(cp_wo0())
        for n in range(REP // 2):
            q_item(0, 0, n, 0)
        wait(cp_wq0(1))
        start(cp_x(5, NT - 5, 4))
        for n in range(REP // 2, REP):
            q_item(0, 0, n, 0)
        wait(cp_x(1, 1, 1))
        for ci in range(REP):
            pre_chunk(1, ci)
        wait(cp_kv0())
        transpose_k(0)
        wait(cp_x(2, 1, 2))

        reset_tokens()
        step(0, 0, do_o=False, pre_t=2)
        wait(cp_wo0())
        wait(cp_x(3, 2, 3))
        start(cp_rest())
        start(cp_wm_b())
        start(cp_ff())

        def body_a0(i, carry):
            j = 2 * i + 1

            @pl.when(i == 1)
            def _():
                wait(cp_x(5, NT - 5, 4))

            reset_tokens()
            step(j, 1, pre_t=j + 2)
            step(j + 1, 0, pre_t=jnp.minimum(j + 3, NT - 1))
            return carry

        lax.fori_loop(0, NT // 2 - 1, body_a0, 0)

        wait(cp_rest())
        wait(cp_wm_b())
        for g in range(1, HKV):
            transpose_k(g)

        def body_a1(i, carry):
            j = 2 * i + 1
            reset_tokens()
            j0 = NT - 1
            step(j, 1, mod_p=jnp.minimum(j - j0, 4 * NP - 1))
            step(j + 1, 0, mod_p=jnp.minimum(j + 1 - j0, 4 * NP - 1))
            return carry

        JB = (HKV - 1) * NT + 1
        lax.fori_loop(NT // 2 - 1, (JB - 1) // 2, body_a1, 0)

        def body_b(i, carry):
            j = 2 * i + 1
            t = j - JB - 1
            reset_tokens()
            step(j, 1, fin=True, post_t=jnp.maximum(t, 0))
            step(j + 1, 0, fin=True, post_t=t + 1)

            @pl.when(t >= 0)
            def _():
                start(cp_out(t))
            start(cp_out(t + 1))
            return carry

        lax.fori_loop((JB - 1) // 2, (NS - 2) // 2, body_b, 0)

        reset_tokens()
        parts = []
        step(NS - 1, 1, do_q=False, fin=True, post_t=NT - 3, amax=((NT - 3) * TQ, parts))
        start(cp_out(NT - 3))
        for n in range(NP):
            reset_tokens()
            o_item(HKV - 1, NT - 1, n, 1, True)
            post_chunk(NT - 2, n)
        start(cp_out(NT - 2))
        parts.append(best_rows((NT - 3) * TQ, 2 * TQ))
        av, ai = combine_best(parts)
        reset_tokens()
        for ci in range(REP):
            post_chunk(NT - 1, ci)
        start(cp_out(NT - 1))
        bv, bi = best_rows((NT - 1) * TQ, TQ)
        upd = bv > av
        bv, bi = jnp.where(upd, bv, av), jnp.where(upd, bi, ai)

        rmax = jnp.max(bv, axis=0, keepdims=True)
        idx = jnp.minimum(jnp.min(jnp.where(bv == rmax, bi, S), axis=0, keepdims=True), S - 1)[0, 0]
        base = pl.multiple_of((idx // 16) * 16, 16)
        x1g = acc_v[pl.ds(base, 16), 0:D]
        h2f = ln2(x1g)
        h2g = h2f.astype(BF)
        wait(cp_ff())
        acts = []
        for n in range(F // 128):
            fs = slice(n * 128, (n + 1) * 128)
            gt = jnp.dot(h2g, wg_v[:, fs], preferred_element_type=F32).astype(BF).astype(F32)
            up = jnp.dot(h2g, wu_v[:, fs], preferred_element_type=F32).astype(BF).astype(F32)
            acts.append(((gt * jax.nn.sigmoid(gt)).astype(BF).astype(F32) * up).astype(BF))
        ys = [jnp.dot(acts[n], wd_v[n * 128:(n + 1) * 128, 0:D], preferred_element_type=F32)
              for n in range(F // 128)]
        y = _tree_sum(ys).astype(BF).astype(F32)
        rs = jax.nn.sigmoid(rmax[:, 0:1]).astype(BF).astype(F32)
        y = (y * rs).astype(BF).astype(F32)
        sel = lax.broadcasted_iota(jnp.int32, (16, 1), 0) == (idx - base)
        hb = jnp.where(sel, h2f + y, h2f)
        og = (x1g + mod_row(5) * hb).astype(BF)
        for t in range(NT):
            wait(cp_out(t))
        out_v[pl.ds(base, 16), 0:D] = og
        fin = mk(out_v.at[pl.ds(base, 16), pl.ds(0, D)], out_hbm.at[pl.ds(base, 16)], sem_out.at[0])
        fin.start()
        fin.wait()

    return kernel


def _build():

    @jax.jit
    def fn(A_x, A_k_cache, A_v_cache, A_wq, A_wo, B_x, B_w_r, B_w_gate, B_w_up, B_w_down, c, w_mod):
        x = A_x.reshape(S, D)
        k = A_k_cache.reshape(HKV, SK, DH)
        v = A_v_cache.reshape(HKV, SK, DH)
        any_spec = pl.BlockSpec(memory_space=pl.ANY)
        out = pl.pallas_call(
            _make_kernel(),
            out_shape=jax.ShapeDtypeStruct((S, D), BF),
            in_specs=[any_spec] * 11,
            out_specs=any_spec,
            scratch_shapes=[
                pltpu.VMEM((S, D), BF),
                pltpu.VMEM((HKV, W, DH), BF),
                pltpu.VMEM((HKV, W, DH), BF),
                pltpu.VMEM((HKV, W // 128, DH, 128), BF),
                pltpu.VMEM((D, HQ * DH), BF),
                pltpu.VMEM((HQ * DH, D + 128), BF),
                pltpu.VMEM((D, F), BF),
                pltpu.VMEM((D, F), BF),
                pltpu.VMEM((F, D), BF),
                pltpu.VMEM((D, 4 * D), BF),
                pltpu.VMEM((S, D), BF),
                pltpu.VMEM((S, D), F32),
                pltpu.VMEM((S, D), BF),
                pltpu.VMEM((S, 128), F32),
                pltpu.VMEM((2, REP, TQ, DH), BF),
                pltpu.VMEM((2, REP, TQ, DH), BF),
                pltpu.VMEM((16, 6 * D), F32),
                pltpu.VMEM((8, 128), U32),
                pltpu.VMEM((1, D), F32),
                pltpu.VMEM((D, 128), F32),
                pltpu.VMEM((1, D), BF),
                pltpu.VMEM((D,), BF),
                pltpu.SemaphoreType.DMA((5,)),
                pltpu.SemaphoreType.DMA((5,)),
                pltpu.SemaphoreType.DMA((5,)),
                pltpu.SemaphoreType.DMA((3,)),
                pltpu.SemaphoreType.DMA((1,)),
            ],
            compiler_params=pltpu.CompilerParams(vmem_limit_bytes=110 * 1024 * 1024),
        )(c, B_w_r, x, k, v, A_wq, A_wo, B_w_gate, B_w_up, B_w_down, w_mod)
        return out.reshape(1, S, D)

    return fn


def build():
    return _build()


_IMPL = build()


@jax.jit
def pallas_adaLN_cond__sliding_block_cached__moe_arch_mod__prompt_kernel(
    A_x: jax.Array,
    A_k_cache: jax.Array,
    A_v_cache: jax.Array,
    A_wq: jax.Array,
    A_wo: jax.Array,
    B_x: jax.Array,
    B_w_r: jax.Array,
    B_w_gate: jax.Array,
    B_w_up: jax.Array,
    B_w_down: jax.Array,
    c: jax.Array,
    w_mod: jax.Array,
):
    return _IMPL(A_x, A_k_cache, A_v_cache, A_wq, A_wo, B_x, B_w_r, B_w_gate, B_w_up, B_w_down, c, w_mod)
```

```python
import jax
import jax.numpy as jnp
from jax import lax
import jax.experimental.pallas as pl
import jax.experimental.pallas.tpu as pltpu

S, D, HQ, HKV, DH, SK, F = 2048, 1024, 32, 4, 128, 2048, 3584
W = min(4096, max(256, SK // 4))
REP = HQ // HKV
GW = REP * DH
NP = D // 128
TQ = 128
NT = S // TQ
NS = NT * HKV
CH = TQ // REP
NSP = 11
EPS = 1e-5
BF = jnp.bfloat16
F32 = jnp.float32
U32 = jnp.uint32
LOG2E = 1.4426950408889634
QSCALE = DH ** -0.5 * LOG2E


def _ln(xf, rel=None):
    m = jnp.sum(xf, axis=-1, keepdims=True)
    if rel is not None:
        m = m + rel
    m = m * (1.0 / D)
    d = xf - m
    v = jnp.sum(d * d, axis=-1, keepdims=True) * (1.0 / D)
    return d * lax.rsqrt(v + EPS)


def _recip(l):
    r = pl.reciprocal(l, approx=True)
    return r * (2.0 - l * r)


def _tree_sum(xs):
    while len(xs) > 1:
        xs = [xs[i] + xs[i + 1] if i + 1 < len(xs) else xs[i] for i in range(0, len(xs), 2)]
    return xs[0]


def _make_kernel():
    def kernel(c_ref, wr_ref, x_hbm, k_hbm, v_hbm, wq_hbm, wo_hbm, wg_hbm, wu_hbm, wd_hbm, wm_hbm,
               out_hbm,
               x_v, k_v, v_v, kt_v, wq_v, wo_v, wg_v, wu_v, wd_v, wm_v, out_v, acc_v, h_v, r_v,
               q_s, o_s, mod_v, zero_s, wr_s, csb_v, c_v, wrb_v, act_v,
               sem_x, sem_wm, sem_g0, sem_rest, sem_out):
        mk = pltpu.make_async_copy

        def cp_x(t0, n, s):
            return [mk(x_hbm.at[pl.ds(t0 * TQ, n * TQ)], x_v.at[pl.ds(t0 * TQ, n * TQ), pl.ds(0, D)], sem_x.at[s])]

        def cp_wm(c0, n, s):
            return [mk(wm_hbm.at[:, pl.ds(c0, n)], wm_v.at[:, pl.ds(c0 % (4 * D), n)], sem_wm.at[s])]

        def cp_wq0(half):
            c0 = half * (GW // 2)
            return [mk(wq_hbm.at[:, pl.ds(c0, GW // 2)], wq_v.at[:, pl.ds(c0, GW // 2)], sem_g0.at[half])]

        def cp_kv0():
            return [mk(k_hbm.at[0, pl.ds(SK - W, W), :], k_v.at[0], sem_g0.at[2]),
                    mk(v_hbm.at[0, pl.ds(SK - W, W), :], v_v.at[0], sem_g0.at[3])]

        def cp_wo0():
            return [mk(wo_hbm.at[pl.ds(0, GW)], wo_v.at[pl.ds(0, GW), pl.ds(0, D)], sem_g0.at[4])]

        def cp_rest():
            n = HKV - 1
            return [mk(wq_hbm.at[:, pl.ds(GW, n * GW)], wq_v.at[:, pl.ds(GW, n * GW)], sem_rest.at[0]),
                    mk(wo_hbm.at[pl.ds(GW, n * GW)], wo_v.at[pl.ds(GW, n * GW), pl.ds(0, D)], sem_rest.at[0]),
                    mk(k_hbm.at[pl.ds(1, n), pl.ds(SK - W, W), :], k_v.at[pl.ds(1, n)], sem_rest.at[0]),
                    mk(v_hbm.at[pl.ds(1, n), pl.ds(SK - W, W), :], v_v.at[pl.ds(1, n)], sem_rest.at[0])]

        def cp_wm_b():
            return cp_wm(2 * D, 2 * D, 4) + cp_wm(4 * D, 2 * D, 4)

        def cp_ff():
            return [mk(wg_hbm, wg_v, sem_rest.at[1]), mk(wu_hbm, wu_v, sem_rest.at[1]), mk(wd_hbm, wd_v, sem_rest.at[1])]

        def cp_out(t):
            r0 = t * TQ if isinstance(t, int) else pl.multiple_of(t * TQ, TQ)
            return [mk(out_v.at[pl.ds(r0, TQ), pl.ds(0, D)], out_hbm.at[pl.ds(r0, TQ)], sem_out.at[0])]

        def start(cps):
            for cp in cps:
                cp.start()

        def wait(cps):
            for cp in cps:
                cp.wait()

        def rows(r0, n):
            return pl.ds(r0 if isinstance(r0, int) else pl.multiple_of(r0, n), n)

        state = {"dead": [], "rel": None}

        def tok(v):
            u = pltpu.bitcast(v[0:16, 0:128] if v.dtype == BF else v[0:8, 0:128], U32)
            return u & zero_s[...]

        def take_rel():
            if state["rel"] is None:
                return None
            return jnp.concatenate([pltpu.bitcast(state["rel"], F32)[:, 0:1]] * (CH // 8), axis=0)

        def with_dead(lhs):
            ready = [z for (z, n) in state["dead"] if n <= 0]
            state["dead"] = [(z, n - 1) for (z, n) in state["dead"] if n > 0]
            if not ready:
                return lhs
            z = ready[0]
            for z2 in ready[1:]:
                z = z | z2
            n = lhs.shape[0]
            last = pltpu.bitcast(pltpu.bitcast(lhs[n - 16:n, :], U32) | z, BF)
            return jnp.concatenate([lhs[0:n - 16, :], last], axis=0)

        def reset_tokens():
            state["dead"] = []
            state["rel"] = None

        def cs_dot(cs16, c0, n):
            ps = [jnp.dot(cs16[:, k * 128:(k + 1) * 128], wm_v[k * 128:(k + 1) * 128, c0:c0 + n],
                          preferred_element_type=F32) for k in range(NP)]
            return _tree_sum(ps).astype(BF).astype(F32)

        def mod_row(which):
            return mod_v[0:1, which * D:(which + 1) * D]

        def one_plus(which):
            return (1 + mod_row(which).astype(BF)).astype(F32)

        def pre_chunk(t, ci):
            sl = rows(t * TQ + ci * CH, CH)
            h = (_ln(x_v[sl, 0:D].astype(F32), take_rel()) * one_plus(1) + mod_row(0)).astype(BF)
            h_v[sl, 0:D] = h
            state["dead"].append((tok(h[CH - 16:CH, D - 128:D]), 0))

        def ln2(x1, rel=None):
            return _ln(x1, rel) * one_plus(4) + mod_row(3)

        def post_chunk(t, ci):
            sl = rows(t * TQ + ci * CH, CH)
            x1 = acc_v[sl, 0:D]
            h2 = ln2(x1, take_rel())
            r = jnp.sum(h2 * wr_s[...], axis=-1, keepdims=True).astype(BF).astype(F32)
            ob = (x1 + mod_row(5) * h2).astype(BF)
            out_v[sl, 0:D] = ob
            r_v[sl, :] = jnp.broadcast_to(r, (CH, 128))
            state["dead"].append((tok(ob[CH - 16:CH, D - 128:D]) | tok(jnp.broadcast_to(r[CH - 8:CH, :], (8, 128))), 1))

        def mod_chunk(p, ci, acc):
            c0 = pl.multiple_of(p * 128, 128)
            ks = slice(ci * 128, (ci + 1) * 128)
            prod = wm_v[ks, pl.ds(c0, 128)].astype(F32) * csb_v[ks, :]
            part = _tree_sum([prod[i * 8:(i + 1) * 8, :] for i in range(16)])
            acc = part if acc is None else acc + part
            if ci == REP - 1:
                tot = jnp.sum(acc, axis=0, keepdims=True).astype(BF).astype(F32)
                dst = pl.multiple_of(jnp.where(c0 >= 2 * D, c0, c0 + 4 * D), 128)
                mod_v[0:8, pl.ds(dst, 128)] = jnp.broadcast_to(tot, (8, 128))
            state["dead"].append((tok(acc), 0))
            return acc

        def q_item(gq, tq, n, slot):
            c0 = gq * GW + n * DH
            if not isinstance(c0, int):
                c0 = pl.multiple_of(c0, DH)
            q = jnp.dot(h_v[rows(tq * TQ, TQ), 0:D], wq_v[:, pl.ds(c0, DH)], preferred_element_type=F32)
            q_s[slot, n] = (q * QSCALE).astype(BF)

        def o_item(go, to, n, slot, fin, dead=False):
            oo = jnp.concatenate([with_dead(o_s[slot, k]) if (dead and k == 0) else o_s[slot, k] for k in range(REP)], axis=1)
            cs_ = slice(n * 128, (n + 1) * 128)
            part = jnp.dot(oo, wo_v[rows(go * GW, GW), cs_], preferred_element_type=F32)
            sl = rows(to * TQ, TQ)
            if fin:
                ga = mod_v[0:1, 2 * D + n * 128:2 * D + (n + 1) * 128]
                acc_v[sl, cs_] = x_v[sl, cs_].astype(F32) + ga * (acc_v[sl, cs_] + part)
            else:
                acc_v[sl, cs_] += part

        def s_item(g, hh, slot):
            qq = with_dead(q_s[slot, hh])
            return jnp.concatenate([jnp.dot(qq, kt_v[g, n], preferred_element_type=F32)
                                    for n in range(W // 128)], axis=1)

        def softmax_item(s):
            m = jnp.max(s, axis=-1, keepdims=True)
            p = jnp.exp2(s - m)
            l = jnp.sum(p, axis=-1, keepdims=True)
            return p.astype(BF), _recip(l)

        def pv_item(g, hh, slot, p, rl):
            o = jnp.dot(p, v_v[g], preferred_element_type=F32)
            state["rel"] = tok(o)
            o_s[slot, hh] = (o * rl).astype(BF)

        def step(j, slot, do_q=True, do_o=True, fin=False, pre_t=None, post_t=None, mod_p=None, amax=None):
            g = j // NT
            gq, tq = (j + 1) // NT, (j + 1) % NT
            go, to = (j - 1) // NT, (j - 1) % NT
            s_next = s_item(g, 0, slot)
            macc = None
            for hh in range(REP):
                s_cur = s_next
                if hh + 1 < REP:
                    s_next = s_item(g, hh + 1, slot)
                if do_q:
                    q_item(gq, tq, hh, 1 - slot)
                if pre_t is not None:
                    pre_chunk(pre_t, hh)
                if post_t is not None:
                    post_chunk(post_t, hh)
                if mod_p is not None:
                    macc = mod_chunk(mod_p, hh, macc)
                if amax is not None:
                    n_ = amax[0] // REP
                    amax[1].append(best_rows(hh * n_, n_))
                    state["dead"].append((tok(amax[1][-1][0]) | tok(pltpu.bitcast(amax[1][-1][1], F32)), 0))
                p, rl = softmax_item(s_cur)
                if do_o:
                    o_item(go, to, hh, 1 - slot, fin)
                pv_item(g, hh, slot, p, rl)

        def winner(bv, bi):
            rmax = jnp.max(bv, axis=0, keepdims=True)
            idx = jnp.minimum(jnp.min(jnp.where(bv == rmax, bi, S), axis=0, keepdims=True), S - 1)[0, 0]
            return rmax, idx, pl.multiple_of((idx // 16) * 16, 16)

        def gate_up(h2g, n):
            fs = slice(n * 128, (n + 1) * 128)
            gt = jnp.dot(h2g, wg_v[:, fs], preferred_element_type=F32).astype(BF).astype(F32)
            up = jnp.dot(h2g, wu_v[:, fs], preferred_element_type=F32).astype(BF).astype(F32)
            return ((gt * jax.nn.sigmoid(gt)).astype(BF).astype(F32) * up).astype(BF)

        def transpose_k(g):
            for n in range(W // 128):
                kt_v[g, n] = k_v[g, n * 128:(n + 1) * 128, :].astype(F32).T.astype(BF)

        def combine_best(items):
            while len(items) > 1:
                nxt = []
                for i in range(0, len(items) - 1, 2):
                    (av, ai), (bv, bi) = items[i], items[i + 1]
                    upd = bv > av
                    nxt.append((jnp.where(upd, bv, av), jnp.where(upd, bi, ai)))
                if len(items) % 2:
                    nxt.append(items[-1])
                items = nxt
            return items[0]

        def best_rows(r0, n):
            sub = lax.broadcasted_iota(jnp.int32, (8, 128), 0)
            return combine_best([(r_v[r0 + i * 8:r0 + (i + 1) * 8, :], sub + (r0 + i * 8)) for i in range(n // 8)])

        cp_small = [mk(c_ref, c_v, sem_rest.at[2]), mk(wr_ref, wrb_v, sem_rest.at[2])]
        start(cp_small)
        start(cp_x(0, 1, 0))
        for ci in range(4):
            start(cp_wm(ci * 512, 512, ci))
        zero_s[...] = jnp.zeros((8, 128), U32)

        def zero_body(i, carry):
            acc_v[pl.ds(pl.multiple_of(i * 128, 128), 128), 0:D] = jnp.zeros((128, D), F32)
            return carry
        lax.fori_loop(0, S // 128, zero_body, 0)
        wait(cp_small)
        cs = c_v[...].astype(F32)
        cs16 = jnp.broadcast_to((cs * jax.nn.sigmoid(cs)).astype(BF), (16, D))
        wr_s[...] = wrb_v[...].astype(F32).reshape(1, D)
        csb_v[...] = jnp.broadcast_to(cs16[0:1, :].astype(F32), (128, D)).T
        wait(cp_x(0, 1, 0))
        start(cp_wq0(0))
        start(cp_wq0(1))
        start(cp_x(1, 1, 1))
        start(cp_kv0())
        start(cp_x(2, 1, 2))
        for ci in range(4):
            wait(cp_wm(ci * 512, 512, ci))
            mod_v[:, ci * 512:(ci + 1) * 512] = cs_dot(cs16, ci * 512, 512)
        reset_tokens()
        for ci in range(REP):
            pre_chunk(0, ci)
        reset_tokens()
        wait(cp_wq0(0))
        start(cp_x(3, 2, 3))
        start(cp_wo0())
        for n in range(REP // 2):
            q_item(0, 0, n, 0)
        wait(cp_wq0(1))
        start(cp_x(5, NT - 5, 4))
        for n in range(REP // 2, REP):
            q_item(0, 0, n, 0)
        wait(cp_x(1, 1, 1))
        for ci in range(REP):
            pre_chunk(1, ci)
        wait(cp_kv0())
        transpose_k(0)
        wait(cp_x(2, 1, 2))

        reset_tokens()
        step(0, 0, do_o=False, pre_t=2)
        wait(cp_wo0())
        wait(cp_x(3, 2, 3))
        start(cp_rest())
        start(cp_wm_b())
        start(cp_ff())

        def body_a0(i, carry):
            j = 2 * i + 1

            @pl.when(i == 1)
            def _():
                wait(cp_x(5, NT - 5, 4))

            reset_tokens()
            step(j, 1, pre_t=j + 2)
            step(j + 1, 0, pre_t=jnp.minimum(j + 3, NT - 1))
            return carry

        lax.fori_loop(0, NT // 2 - 1, body_a0, 0)

        wait(cp_rest())
        wait(cp_wm_b())
        for g in range(1, HKV):
            transpose_k(g)

        def body_a1(i, carry):
            j = 2 * i + 1
            reset_tokens()
            j0 = NT - 1
            step(j, 1, mod_p=jnp.minimum(j - j0, 4 * NP - 1))
            step(j + 1, 0, mod_p=jnp.minimum(j + 1 - j0, 4 * NP - 1))
            return carry

        JB = (HKV - 1) * NT + 1
        lax.fori_loop(NT // 2 - 1, (JB - 1) // 2, body_a1, 0)

        def body_b(i, carry):
            j = 2 * i + 1
            t = j - JB - 1
            reset_tokens()
            step(j, 1, fin=True, post_t=jnp.maximum(t, 0))
            step(j + 1, 0, fin=True, post_t=t + 1)

            @pl.when(t >= 0)
            def _():
                start(cp_out(t))
            start(cp_out(t + 1))
            return carry

        lax.fori_loop((JB - 1) // 2, (NS - 2) // 2, body_b, 0)

        wait(cp_ff())
        reset_tokens()
        parts = []
        step(NS - 1, 1, do_q=False, fin=True, post_t=NT - 3, amax=((NT - 3) * TQ, parts))
        start(cp_out(NT - 3))
        cv, ci_ = combine_best(parts + [best_rows((NT - 3) * TQ, TQ)])
        _, _, base_c = winner(cv, ci_)
        h2c = ln2(acc_v[pl.ds(base_c, 16), 0:D]).astype(BF)
        for n in range(NP):
            reset_tokens()
            if n == NP - 1:
                state["dead"].append((tok(h2c), 0))
            o_item(HKV - 1, NT - 1, n, 1, True, dead=True)
            post_chunk(NT - 2, n)
        start(cp_out(NT - 2))
        av, ai = combine_best([(cv, ci_), best_rows((NT - 2) * TQ, TQ)])
        reset_tokens()
        for ci in range(REP):
            post_chunk(NT - 1, ci)
            for n in range(ci * NSP // REP, (ci + 1) * NSP // REP):
                act_v[:, n * 128:(n + 1) * 128] = gate_up(h2c, n)
        start(cp_out(NT - 1))
        bv, bi = best_rows((NT - 1) * TQ, TQ)
        upd = bv > av
        bv, bi = jnp.where(upd, bv, av), jnp.where(upd, bi, ai)

        rmax, idx, base = winner(bv, bi)
        x1g = acc_v[pl.ds(base, 16), 0:D]
        h2f = ln2(x1g)
        h2g = h2f.astype(BF)

        @pl.when(base != base_c)
        def _():
            for n in range(NSP):
                act_v[:, n * 128:(n + 1) * 128] = gate_up(h2g, n)

        acts = [act_v[:, n * 128:(n + 1) * 128] for n in range(NSP)] + [gate_up(h2g, n) for n in range(NSP, F // 128)]
        ys = [jnp.dot(acts[n], wd_v[n * 128:(n + 1) * 128, :], preferred_element_type=F32)
              for n in range(F // 128)]
        y = _tree_sum(ys).astype(BF).astype(F32)
        rs = jax.nn.sigmoid(rmax[:, 0:1]).astype(BF).astype(F32)
        y = (y * rs).astype(BF).astype(F32)
        sel = lax.broadcasted_iota(jnp.int32, (16, 1), 0) == (idx - base)
        hb = jnp.where(sel, h2f + y, h2f)
        og = (x1g + mod_row(5) * hb).astype(BF)
        for t in range(NT):
            wait(cp_out(t))
        out_v[pl.ds(base, 16), 0:D] = og
        fin = mk(out_v.at[pl.ds(base, 16), pl.ds(0, D)], out_hbm.at[pl.ds(base, 16)], sem_out.at[0])
        fin.start()
        fin.wait()

    return kernel


def _build():

    @jax.jit
    def fn(A_x, A_k_cache, A_v_cache, A_wq, A_wo, B_x, B_w_r, B_w_gate, B_w_up, B_w_down, c, w_mod):
        x = A_x.reshape(S, D)
        k = A_k_cache.reshape(HKV, SK, DH)
        v = A_v_cache.reshape(HKV, SK, DH)
        any_spec = pl.BlockSpec(memory_space=pl.ANY)
        out = pl.pallas_call(
            _make_kernel(),
            out_shape=jax.ShapeDtypeStruct((S, D), BF),
            in_specs=[any_spec] * 11,
            out_specs=any_spec,
            scratch_shapes=[
                pltpu.VMEM((S, D), BF),
                pltpu.VMEM((HKV, W, DH), BF),
                pltpu.VMEM((HKV, W, DH), BF),
                pltpu.VMEM((HKV, W // 128, DH, 128), BF),
                pltpu.VMEM((D, HQ * DH), BF),
                pltpu.VMEM((HQ * DH, D + 128), BF),
                pltpu.VMEM((D, F), BF),
                pltpu.VMEM((D, F), BF),
                pltpu.VMEM((F, D), BF),
                pltpu.VMEM((D, 4 * D), BF),
                pltpu.VMEM((S, D), BF),
                pltpu.VMEM((S, D), F32),
                pltpu.VMEM((S, D), BF),
                pltpu.VMEM((S, 128), F32),
                pltpu.VMEM((2, REP, TQ, DH), BF),
                pltpu.VMEM((2, REP, TQ, DH), BF),
                pltpu.VMEM((16, 6 * D), F32),
                pltpu.VMEM((8, 128), U32),
                pltpu.VMEM((1, D), F32),
                pltpu.VMEM((D, 128), F32),
                pltpu.VMEM((1, D), BF),
                pltpu.VMEM((D,), BF),
                pltpu.VMEM((16, F), BF),
                pltpu.SemaphoreType.DMA((5,)),
                pltpu.SemaphoreType.DMA((5,)),
                pltpu.SemaphoreType.DMA((5,)),
                pltpu.SemaphoreType.DMA((3,)),
                pltpu.SemaphoreType.DMA((1,)),
            ],
            compiler_params=pltpu.CompilerParams(vmem_limit_bytes=110 * 1024 * 1024),
        )(c, B_w_r, x, k, v, A_wq, A_wo, B_w_gate, B_w_up, B_w_down, w_mod)
        return out.reshape(1, S, D)

    return fn


_IMPL = _build()


@jax.jit
def pallas_adaLN_cond__sliding_block_cached__moe_arch_mod__prompt_kernel(
    A_x: jax.Array,
    A_k_cache: jax.Array,
    A_v_cache: jax.Array,
    A_wq: jax.Array,
    A_wo: jax.Array,
    B_x: jax.Array,
    B_w_r: jax.Array,
    B_w_gate: jax.Array,
    B_w_up: jax.Array,
    B_w_down: jax.Array,
    c: jax.Array,
    w_mod: jax.Array,
):
    return _IMPL(A_x, A_k_cache, A_v_cache, A_wq, A_wo, B_x, B_w_r, B_w_gate, B_w_up, B_w_down, c, w_mod)
```
